```python
import jax
import jax.numpy as jnp

def _softmax(x, axis=-1):
    return jax.nn.softmax(x, axis=axis)

def _gelu(x):
    return jax.nn.gelu(x, approximate=True)

def _silu(x):
    return jax.nn.silu(x)

def _sigmoid(x):
    return jax.nn.sigmoid(x)

def _layernorm(x, axis=-1, eps=1e-05):
    m = jnp.mean(x, axis=axis, keepdims=True)
    v = jnp.var(x, axis=axis, keepdims=True)
    return (x - m) / jnp.sqrt(v + eps)

def _scatter_add(tgt, idx, src, axis=0):
    return tgt.at[idx].add(src)

def _segment_sum(src, seg, n):
    return jax.ops.segment_sum(src, seg, n)

class _Rng:

    def __init__(self, key):
        self._k = key

    def _next(self):
        self._k, sub = jax.random.split(self._k)
        return sub

    def normal(self, shape):
        return jax.random.normal(self._next(), shape, dtype=jnp.bfloat16)

    def randint(self, lo, hi, shape):
        return jax.random.randint(self._next(), shape, lo, hi, dtype=jnp.int32)

    def uniform(self, shape, lo=0.0, hi=1.0):
        return jax.random.uniform(self._next(), shape, jnp.bfloat16, lo, hi)

    def permutation(self, n):
        return jax.random.permutation(self._next(), n)
kernel_name = 'concat_heads__memory_aug_recurrent_mem_tr__sliding_local_dilated__prompt'

def setup_inputs():
    _rng = _Rng(jax.random.key(int.from_bytes(__import__("os").urandom(4), "little")))
    _w = lambda a: (lambda t: t.astype(jnp.bfloat16) if jnp.issubdtype(t.dtype, jnp.floating) else t)(jnp.asarray(a))

    def _A_setup():
        B, S, Dm = (1, 2048, 1024)
        H, Dh = (32, 128)
        M, seg = (8, 32)
        seg = min(seg, S)
        S = S // seg * seg
        return {'x': _w((lambda *s: _rng.normal(s) * 0.05)(B, S, Dm)), 'mem0': _w((lambda *s: _rng.normal(s) * 0.05)(B, M, Dm)), 'Wq': _w((lambda *s: _rng.normal(s) * 0.05)(Dm, H, Dh) * Dm ** (-0.5)), 'Wk': _w((lambda *s: _rng.normal(s) * 0.05)(Dm, H, Dh) * Dm ** (-0.5)), 'Wv': _w((lambda *s: _rng.normal(s) * 0.05)(Dm, H, Dh) * Dm ** (-0.5)), 'Wo': _w((lambda *s: _rng.normal(s) * 0.05)(H, Dh, Dm) * (H * Dh) ** (-0.5)), 'seg_len': seg}
    _A_in = _A_setup()

    def _B_setup():
        B, S, D = (1, 2048, 1024)
        return {'x': _w((lambda *s: _rng.normal(s) * 0.05)(B, S, D)), 'wqkv': _w((lambda *s: _rng.normal(s) * 0.05)(D, 3 * D)), 'wo': _w((lambda *s: _rng.normal(s) * 0.05)(D, D))}
    _B_in = _B_setup()
    return {'A_x': _A_in['x'], 'A_mem0': _A_in['mem0'], 'A_Wq': _A_in['Wq'], 'A_Wk': _A_in['Wk'], 'A_Wv': _A_in['Wv'], 'A_Wo': _A_in['Wo'], 'A_seg_len': _A_in['seg_len'], 'B_x': _B_in['x'], 'B_wqkv': _B_in['wqkv'], 'B_wo': _B_in['wo']}

def reference(A_x, A_mem0, A_Wq, A_Wk, A_Wv, A_Wo, A_seg_len, B_x, B_wqkv, B_wo):

    def _A_ref(x, mem0, Wq, Wk, Wv, Wo, seg_len):
        B, S, Dm = x.shape
        H, Dh = (Wq.shape[1], Wq.shape[2])
        M = mem0.shape[1]
        scale = Dh ** (-0.5)
        n_seg = S // seg_len
        L = M + seg_len
        idx = jnp.arange(L)
        mask = (idx[:, None] < M) | (idx[:, None] >= idx[None, :])
        mem = mem0
        outs = []
        for s in range(n_seg):
            xs = x[:, s * seg_len:(s + 1) * seg_len, :].copy()
            h = jnp.concatenate([mem, xs], axis=1)
            q = jnp.einsum('btd,dhe->bhte', h, Wq)
            k = jnp.einsum('btd,dhe->bhte', h, Wk)
            v = jnp.einsum('btd,dhe->bhte', h, Wv)
            scores = jnp.einsum('bhqe,bhke->bhqk', q, k) * scale
            scores = jnp.where(mask[None, None], scores, -1000000000.0)
            p = _softmax(scores, axis=-1)
            o = jnp.einsum('bhqk,bhke->bhqe', p, v)
            o = jnp.einsum('bhte,hed->btd', o, Wo)
            mem = o[:, :M, :].copy()
            outs.append(o[:, M:, :])
        return jnp.concatenate(outs, axis=1)

    def _B_ref(x, wqkv, wo):
        B, S, D = x.shape
        H = 32
        Dh = D // H
        W, dil = (8, 2)
        qkv = (lambda x, *d: x.transpose(*d))((x @ wqkv).reshape(B, S, 3, H, Dh), 2, 0, 3, 1, 4)
        q, k, v = (qkv[0], qkv[1], qkv[2])
        scale = Dh ** (-0.5)
        pos = jnp.arange(S)
        off = jnp.arange(W) * dil
        idx = pos[:, None] - off[None, :]
        mask = idx >= 0
        idx_c = jnp.where(mask, idx, 0).reshape(-1)
        kg = k[:, :, idx_c, :].reshape(B, H, S, W, Dh)
        vg = v[:, :, idx_c, :].reshape(B, H, S, W, Dh)
        logits = jnp.einsum('bhsd,bhswd->bhsw', q, kg) * scale
        logits = jnp.where(mask[None, None, :, :], logits, -1000000000.0)
        attn = _softmax(logits, axis=-1)
        o = jnp.einsum('bhsw,bhswd->bhsd', attn, vg)
        return (lambda x, *d: x.transpose(*d))(o, 0, 2, 1, 3).reshape(B, S, D) @ wo
    a = _A_ref(A_x, A_mem0, A_Wq, A_Wk, A_Wv, A_Wo, A_seg_len)
    b = _B_ref(B_x, B_wqkv, B_wo)
    return jnp.concatenate([a, b], axis=-1)
```

```python
import functools

import jax
import jax.numpy as jnp
import jax.experimental.pallas as pl
import jax.experimental.pallas.tpu as pltpu

_NT = (((1,), (1,)), ((), ()))
_MASKED = -1000000000.0

_HB, _W, _DIL = 32, 8, 2
_T = 64
_PAD = 16
_OFFS = (-1, 0, 2, 3)
_SQUEEZE = 0.94


def _split(a, b):
    u = jnp.concatenate([a, b], axis=0)
    lo = pltpu.bitcast(u << 16, jnp.float32).astype(jnp.bfloat16)
    hi = pltpu.bitcast(u & jnp.uint32(0xFFFF0000), jnp.float32).astype(jnp.bfloat16)
    return pltpu.bitcast(lo, jnp.uint32), pltpu.bitcast(hi, jnp.uint32)


def _bf16(u):
    return pltpu.bitcast(u, jnp.bfloat16)


def _make_kernel(S, DM, H, DH, M, SEG):
    L = M + SEG
    T, PAD, W, DIL = _T, _PAD, _W, _DIL
    NG = T // 8
    NBLK = S // T
    NCHUNK = NBLK // 2
    NPAIR = H // 2
    assert NCHUNK == NPAIR and DM == 1024 and DH == 128 and DM // _HB == 32
    scale_a = DH ** -0.5
    scale_b = (DM // _HB) ** -0.5

    def kernel(xa_hbm, mem_hbm, wq_hbm, wk_hbm, wv_hbm, woa_hbm, xb_hbm, wb_hbm, wob_hbm,
               out_hbm,
               xa, memv, wa, woa, xb, wb, wob,
               q0, k0, v0, q1, k1, v1, ob0, ob1, outa, outb, hbuf, obuf, acc,
               s_wb, s_misc, s_xb, s_xa, s_pair, s_woa, s_out):
        u32 = lambda r: r.bitcast(jnp.uint32)
        xa_h, woa_h, xb_h, wb_h, wob_h, out_h = (
            u32(xa_hbm), u32(woa_hbm), u32(xb_hbm), u32(wb_hbm), u32(wob_hbm), u32(out_hbm))
        wa_h = [u32(wq_hbm), u32(wk_hbm), u32(wv_hbm)]

        def rows(i, n):
            return pl.ds(i * n, n) if isinstance(i, int) else pl.ds(pl.multiple_of(i * n, n), n)

        def cp_wb(m):
            cols = pl.ds(m * DM, DM)
            return pltpu.make_async_copy(wb_h.at[:, cols], wb.at[:, cols], s_wb.at[m])

        def cp_wob():
            return [pltpu.make_async_copy(wob_h.at[:, e, :, dp, :], wob.at[pl.ds(2 * (2 * dp + e), 2)], s_misc.at[0])
                    for dp in range(16) for e in range(2)]

        def cp_mem():
            return pltpu.make_async_copy(mem_hbm, memv, s_misc.at[1])

        def cp_xb(c):
            return pltpu.make_async_copy(xb_h.at[rows(c, T)], xb.at[rows(c, T)], s_xb.at[c])

        def cp_xa(c):
            return pltpu.make_async_copy(xa_h.at[rows(c, T)], xa.at[rows(c, T)], s_xa.at[c])

        def cp_woa(c):
            return pltpu.make_async_copy(woa_h.at[rows(c, DH)], woa.at[rows(c, DH)], s_woa.at[c])

        def cp_pair(hp):
            return [pltpu.make_async_copy(wa_h[m].at[:, e, :, hp, :],
                                          wa.at[2 * hp + e, :, :, pl.ds(m * DH, DH)], s_pair.at[hp])
                    for m in range(3) for e in range(2)]

        def cp_outb(c):
            return pltpu.make_async_copy(outb.at[rows(c, T)], out_h.at[rows(c, T), pl.ds(DM, DM)], s_out.at[1])

        def cp_outa(s):
            n = SEG // 2
            return pltpu.make_async_copy(outa.at[rows(s, n)], out_h.at[rows(s, n), pl.ds(0, DM)], s_out.at[0])

        def start_a(c):
            for cp in cp_pair(c):
                cp.start()
            cp_woa(c).start()
            cp_xa(c).start()

        cp_xb(0).start()
        for m in range(3):
            cp_wb(m).start()
        cp_xb(1).start()
        for cp in cp_wob():
            cp.start()
        cp_mem().start()

        lane = jax.lax.broadcasted_iota(jnp.int32, (8, 128), 1)

        def permute_wb(m):
            bits = [(b, (lane & (4 * b)) != 0) for b in (1, 2, 4)]
            last = 32 * (lane & 3) + (lane & 28) + (lane >> 5)

            def body(r, carry):
                rs = rows(r, 8)
                t = [wb[rs, pl.ds(m * DM + j * 128, 128)] for j in range(8)]
                if m == 2:
                    t = [t[0]] + [jnp.take_along_axis(t[j], lane ^ (4 * j), axis=1) for j in range(1, 8)]
                for b, bit in bits:
                    t = [jnp.where(bit, t[j ^ b], t[j]) for j in range(8)]
                for j in range(8):
                    wb[rs, pl.ds(m * DM + j * 128, 128)] = jnp.take_along_axis(t[j], last ^ (4 * j), axis=1)
                return carry

            jax.lax.fori_loop(0, DM // 16, body, 0, unroll=8)

        def split_wob():
            def body(dp, carry):
                for r in range(2):
                    a, b = _split(wob[4 * dp + r], wob[4 * dp + 2 + r])
                    wob[4 * dp + r] = a
                    wob[4 * dp + 2 + r] = b
                return carry

            jax.lax.fori_loop(0, 16, body, 0, unroll=4)

        def split_wa(hp, r):
            a, b = _split(wa[2 * hp, r], wa[2 * hp + 1, r])
            wa[2 * hp, r] = a
            wa[2 * hp + 1, r] = b

        B0, B1 = (q0, k0, v0), (q1, k1, v1)

        def proj_tile(blk, bufs, j):
            q, k, v = bufs
            val = jnp.dot(_bf16(xb[rows(blk, T // 2), :]), _bf16(wb[:, j * 128:(j + 1) * 128]),
                          preferred_element_type=jnp.float32)
            if j < 8:
                q[j] = val
            elif j < 16:
                k[j - 8, PAD:PAD + T, :] = val
            else:
                v[j - 16, PAD:PAD + T, :] = val
            return val[0:8]

        def out_tile(blk, ob, j):
            r = jnp.dot(_bf16(ob[...]), _bf16(wob[:, :, j * 128:(j + 1) * 128].reshape(DM // 2, 128)),
                        preferred_element_type=jnp.float32)
            outb[rows(blk, T // 2), j * 128:(j + 1) * 128] = pltpu.bitcast(r.astype(jnp.bfloat16), jnp.uint32)
            return r[0:8]

        def attn_pieces(blk, bufs, ob):
            q, k, v = bufs
            sub = jax.lax.broadcasted_iota(jnp.int32, (8, 128), 0)
            never = (blk + sub) < 0
            st = {}

            def gate(a, tok):
                return a if tok is None else jnp.where(never, tok, a)

            def win(g, w):
                return pl.ds(PAD + g * 8 - DIL * w, 8)

            def qk(g, half, tok):
                accs = st.setdefault(("acc", g), [None] * W)
                for j in range(4 * half, 4 * half + 4):
                    qj = gate(q[j, g * 8:g * 8 + 8, :], tok)
                    for w in range(W):
                        p = qj * k[j, win(g, w), :]
                        accs[w] = p if accs[w] is None else accs[w] + p
                if half == 1:
                    lg = []
                    for w in range(W):
                        a = accs[w]
                        a = a + pltpu.roll(a, 64, 1)
                        a = a + pltpu.roll(a, 32, 1)
                        a = a * scale_b
                        if g * 8 < DIL * w:
                            a = jnp.where(blk * T + g * 8 + sub >= DIL * w, a, _MASKED)
                        lg.append(a)
                    m = functools.reduce(jnp.maximum, lg)
                    es = [jnp.exp(a - m) for a in lg]
                    st["e", g] = es
                    st["inv", g] = 1.0 / functools.reduce(jnp.add, es)

            def pv(g, half, tok):
                inv = gate(st["inv", g], tok)
                ps = [e * inv for e in st["e", g]]
                for j in range(4 * half, 4 * half + 4):
                    st["o", g, j] = functools.reduce(jnp.add, [ps[w] * v[j, win(g, w), :] for w in range(W)])
                    if g % 2 == 1:
                        pair = jnp.concatenate([st.pop(("o", g - 1, j)), st.pop(("o", g, j))], axis=0)
                        ob[(g // 2) * 8:(g // 2) * 8 + 8, j * 128:(j + 1) * 128] = pltpu.bitcast(
                            pair.astype(jnp.bfloat16), jnp.uint32)

            sched = {}
            for g in range(NG):
                for n, (fn, half) in enumerate([(qk, 0), (qk, 1), (pv, 0), (pv, 1)]):
                    at = max(int((32 // NG * g + _OFFS[n]) * _SQUEEZE), -1)
                    sched.setdefault(at, []).append(functools.partial(fn, g, half))
            return sched

        def phase(blk, cur, nxt, oc, op, do_proj=True, do_attn=True, do_out=True, pair=None):
            if do_proj:
                for j in range(8):
                    nxt[1][j, 0:PAD, :] = cur[1][j, T:T + PAD, :]
                    nxt[2][j, 0:PAD, :] = cur[2][j, T:T + PAD, :]
            sched = attn_pieces(blk, cur, oc) if do_attn else {}
            slots = []
            if do_proj:
                slots += [functools.partial(proj_tile, blk + 1, nxt, j) for j in range(24)]
            if do_out:
                slots += [functools.partial(out_tile, blk - 1, op, j) for j in range(8)]
            for f in sched.pop(-1, []):
                f(None)
            for n, slot in enumerate(slots):
                tok = slot()
                for m in range(n * 32 // len(slots), (n + 1) * 32 // len(slots)):
                    for f in sched.pop(m, []):
                        f(tok)
                    if pair is not None:
                        split_wa(pair, 2 * m)
                        split_wa(pair, 2 * m + 1)
            assert not sched

        cp_xb(0).wait()
        for m in range(3):
            cp_wb(m).wait()
            if m == 1:
                start_a(0)
            permute_wb(m)
            for j in range(8 * m, 8 * m + 8):
                proj_tile(0, B0, j)
        for j in range(8):
            k0[j, 0:PAD, :] = jnp.broadcast_to(k0[j, PAD:PAD + 1, :], (PAD, 128))
            v0[j, 0:PAD, :] = jnp.broadcast_to(v0[j, PAD:PAD + 1, :], (PAD, 128))
        phase(0, B0, B1, ob0, ob1, do_out=False)
        for cp in cp_wob():
            cp.wait()
        split_wob()

        def b_body(i, carry):
            @pl.when(i + 2 < NCHUNK)
            def _():
                cp_xb(i + 2).start()

            start_a(i + 1)
            cp_xb(i + 1).wait()
            for cp in cp_pair(i):
                cp.wait()
            phase(2 * i + 1, B1, B0, ob1, ob0)
            phase(2 * i + 2, B0, B1, ob0, ob1, pair=i)
            cp_outb(i).start()
            return carry

        jax.lax.fori_loop(0, NCHUNK - 1, b_body, 0)
        for cp in cp_pair(NPAIR - 1):
            cp.wait()
        phase(NBLK - 1, B1, B0, ob1, ob0, do_proj=False)
        phase(NBLK, B0, B1, ob0, ob1, do_proj=False, do_attn=False, pair=NPAIR - 1)
        cp_outb(NCHUNK - 1).start()

        cp_mem().wait()
        for c in range(NCHUNK):
            cp_xa(c).wait()
            cp_woa(c).wait()
        hbuf[0:M, :] = memv[...].astype(jnp.float32)
        row = jax.lax.broadcasted_iota(jnp.int32, (L, 128), 0)
        col = jax.lax.broadcasted_iota(jnp.int32, (L, 128), 1)
        WG = 4

        def a_body(s, carry):
            hbuf[M:L, :] = _bf16(xa[rows(s, SEG // 2), :]).astype(jnp.float32)
            allowed = (row < M) | (row >= col)
            real = col < L
            zpad = jnp.zeros((128 - L, DH), jnp.float32)
            qs, ks, vs, es, ls = {}, {}, {}, {}, {}

            def qkv(h):
                r = jnp.dot(hbuf[...], _bf16(wa[h].reshape(DM // 2, 3 * DH)), preferred_element_type=jnp.float32)
                qs[h] = r[:, 0:DH]
                ks[h] = jnp.concatenate([r[:, DH:2 * DH], zpad], axis=0).astype(jnp.bfloat16)
                vs[h] = jnp.concatenate([r[:, 2 * DH:3 * DH], zpad], axis=0).astype(jnp.bfloat16)

            def scores(h):
                sc = jax.lax.dot_general(qs.pop(h), ks.pop(h), _NT, preferred_element_type=jnp.float32) * scale_a
                sc = jnp.where(allowed, sc, _MASKED)
                sc = jnp.where(real, sc, -jnp.inf)
                e = jnp.exp(sc - jnp.max(sc, axis=1, keepdims=True))
                es[h] = e
                ls[h] = 1.0 / jnp.sum(e, axis=1, keepdims=True)

            def values(h):
                obuf[:, h * DH:(h + 1) * DH] = jnp.dot(
                    es.pop(h), vs.pop(h), preferred_element_type=jnp.float32) * ls.pop(h)

            def project(h):
                r = jnp.dot(obuf[:, h * DH:(h + WG) * DH], _bf16(woa[h * DH // 2:(h + WG) * DH // 2, :]),
                            preferred_element_type=jnp.float32)
                if h == 0:
                    acc[...] = r
                elif h + WG < H:
                    acc[...] += r
                else:
                    r = r + acc[...]
                    hbuf[0:M, :] = r[0:M]
                    outa[rows(s, SEG // 2), :] = pltpu.bitcast(r[M:L].astype(jnp.bfloat16), jnp.uint32)

            for h in range(H):
                qkv(h)
                if h >= 1:
                    scores(h - 1)
                if h >= 2:
                    values(h - 2)
                if h >= 15 and h % WG == 3:
                    project(h - 15)
            scores(H - 1)
            values(H - 2)
            project(H - 3 * WG)
            values(H - 1)
            project(H - 2 * WG)
            project(H - WG)
            cp_outa(s).start()
            return carry

        jax.lax.fori_loop(0, S // SEG, a_body, 0)
        pltpu.make_async_copy(outa, out_h.at[:, pl.ds(0, DM)], s_out.at[0]).wait()
        pltpu.make_async_copy(outb, out_h.at[:, pl.ds(DM, DM)], s_out.at[1]).wait()

    f32, u32 = jnp.float32, jnp.uint32
    qkv_bufs = [pltpu.VMEM((8, T, 128), f32), pltpu.VMEM((8, T + PAD, 128), f32), pltpu.VMEM((8, T + PAD, 128), f32)]
    scratch = [
        pltpu.VMEM((S // 2, DM), u32),
        pltpu.VMEM((M, DM), jnp.bfloat16),
        pltpu.VMEM((H, DM // 16, 8, 3 * DH), u32),
        pltpu.VMEM((H * DH // 2, DM), u32),
        pltpu.VMEM((S // 2, DM), u32),
        pltpu.VMEM((DM // 2, 3 * DM), u32),
        pltpu.VMEM((DM // 16, 8, DM), u32),
        *qkv_bufs, *qkv_bufs,
        pltpu.VMEM((T // 2, DM), u32), pltpu.VMEM((T // 2, DM), u32),
        pltpu.VMEM((S // 2, DM), u32), pltpu.VMEM((S // 2, DM), u32),
        pltpu.VMEM((L, DM), f32), pltpu.VMEM((L, H * DH), f32), pltpu.VMEM((L, DM), f32),
        pltpu.SemaphoreType.DMA((3,)), pltpu.SemaphoreType.DMA((2,)),
        pltpu.SemaphoreType.DMA((NCHUNK,)), pltpu.SemaphoreType.DMA((NCHUNK,)),
        pltpu.SemaphoreType.DMA((NPAIR,)), pltpu.SemaphoreType.DMA((NCHUNK,)),
        pltpu.SemaphoreType.DMA((2,)),
    ]
    return kernel, scratch


def pallas_concat_heads__memory_aug_recurrent_mem_tr__sliding_local_dilated__prompt_kernel(
    A_x, A_mem0, A_Wq, A_Wk, A_Wv, A_Wo, A_seg_len, B_x, B_wqkv, B_wo,
):
    B, S, DM = A_x.shape
    H, DH = A_Wq.shape[1], A_Wq.shape[2]
    M = A_mem0.shape[1]
    assert B == 1 and B_x.shape == (1, S, DM)
    kernel, scratch = _make_kernel(S, DM, H, DH, M, int(A_seg_len))
    heads = lambda w: w.reshape(DM // 16, 2, 8, H, DH)
    out = pl.pallas_call(
        kernel,
        out_shape=jax.ShapeDtypeStruct((S, 2 * DM), jnp.bfloat16),
        in_specs=[pl.BlockSpec(memory_space=pl.ANY)] * 9,
        out_specs=pl.BlockSpec(memory_space=pl.ANY),
        scratch_shapes=scratch,
        compiler_params=pltpu.CompilerParams(vmem_limit_bytes=100 * 1024 * 1024),
    )(
        A_x.reshape(S, DM), A_mem0.reshape(M, DM), heads(A_Wq), heads(A_Wk), heads(A_Wv),
        A_Wo.reshape(H * DH, DM), B_x.reshape(S, DM), B_wqkv,
        B_wo.reshape(_HB // 16, 2, 8, DM // _HB, DM),
    )
    return out.reshape(1, S, 2 * DM)
```

```python
import functools

import jax
import jax.numpy as jnp
import jax.experimental.pallas as pl
import jax.experimental.pallas.tpu as pltpu

_NT = (((1,), (1,)), ((), ()))
_MASKED = -1000000000.0

_HB, _W, _DIL = 32, 8, 2
_PAD = 16
_TB = 256
_WG = 4
_LAG = 15
_TIE = 2
_TIE_R, _TIE_C = 64, 512
_QCH = 4


def _split(a, b):
    u = jnp.concatenate([a, b], axis=0)
    lo = pltpu.bitcast(u << 16, jnp.float32).astype(jnp.bfloat16)
    hi = pltpu.bitcast(u & jnp.uint32(0xFFFF0000), jnp.float32).astype(jnp.bfloat16)
    return pltpu.bitcast(lo, jnp.uint32), pltpu.bitcast(hi, jnp.uint32)


def _bf16(u):
    return pltpu.bitcast(u, jnp.bfloat16)


def _words(x):
    return pltpu.bitcast(x.astype(jnp.bfloat16), jnp.uint32)


def _tie(never, tok, x, r=0, c=0):
    cat = lambda parts, axis: jnp.concatenate([p for p in parts if p.size], axis=axis)
    mid = cat([x[r:r + 8, :c], jnp.where(never, tok, x[r:r + 8, c:c + 128]), x[r:r + 8, c + 128:]], 1)
    return cat([x[:r], mid, x[r + 8:]], 0)


def _rows(i, n):
    return pl.ds(i * n, n) if isinstance(i, int) else pl.ds(pl.multiple_of(i * n, n), n)


def _make_kernel(S, DM, H, DH, M, SEG):
    L = M + SEG
    PAD, W, DIL, TB, WG = _PAD, _W, _DIL, _TB, _WG
    NB = S // TB
    NPAIR = H // 2
    RG = DM // 16
    GPI = RG // NB
    assert DM == 1024 and DH == 128 and DM // _HB == 32 and NPAIR == 2 * NB and PAD >= DIL * (W - 1)
    scale_a = DH ** -0.5
    scale_b = (DM // _HB) ** -0.5

    def kernel(xa_hbm, mem_hbm, wq_hbm, wk_hbm, wv_hbm, woa_hbm, xb_hbm, wb_hbm, wob_hbm,
               out_hbm,
               xa, memv, wa, woa, xb, wb0, wb1, wb2, wob, qkv, ob, outs, hbuf, obuf, acc,
               s_wq, s_wb, s_xb, s_pair, s_bg, s_out):
        u32 = lambda r: r.bitcast(jnp.uint32)
        xa_h, woa_h, xb_h, wb_h, wob_h, out_h = (
            u32(xa_hbm), u32(woa_hbm), u32(xb_hbm), u32(wb_hbm), u32(wob_hbm), u32(out_hbm))
        wa_h = [u32(wq_hbm), u32(wk_hbm), u32(wv_hbm)]
        wb = [wb0, wb1, wb2]

        def cp_wq(c):
            n = RG // _QCH
            return pltpu.make_async_copy(wb_h.at[pl.ds(c * n, n), :, pl.ds(0, DM)], wb0.at[pl.ds(c * n, n)], s_wq.at[c])

        def cp_wb(m, c):
            return pltpu.make_async_copy(wb_h.at[_rows(c, GPI), :, pl.ds(m * DM, DM)], wb[m].at[_rows(c, GPI)],
                                         s_wb.at[(m - 1) * NB + c])

        def cp_xb(c):
            return pltpu.make_async_copy(xb_h.at[_rows(c, TB // 2)], xb.at[_rows(c, TB // 2)], s_xb.at[c])

        def cp_pair(hp):
            return [pltpu.make_async_copy(wa_h[m].at[:, e, :, hp, :],
                                          wa.at[2 * hp + e, :, :, pl.ds(m * DH, DH)], s_pair.at[hp])
                    for m in range(3) for e in range(2)]

        def cp_woa(c):
            n = H * DH // 16
            return pltpu.make_async_copy(woa_h.at[_rows(c, n)], woa.at[_rows(c, n)], s_bg.at[0])

        def cp_xa(c):
            n = S // 2 // NPAIR
            return pltpu.make_async_copy(xa_h.at[_rows(c, n)], xa.at[_rows(c, n)], s_bg.at[1])

        def cp_wob():
            return [pltpu.make_async_copy(wob_h.at[:, e, :, dp, :], wob.at[pl.ds(2 * (2 * dp + e), 2)], s_bg.at[2])
                    for dp in range(16) for e in range(2)]

        def cp_mem():
            return pltpu.make_async_copy(mem_hbm, memv, s_bg.at[3])

        def cp_out(s):
            return pltpu.make_async_copy(outs.at[_rows(s, SEG // 2)], out_h.at[_rows(s, SEG // 2)], s_out.at[0])

        cp_xb(0).start()
        for c in range(_QCH):
            cp_wq(c).start()
        cp_wb(1, 0).start()
        cp_xb(1).start()
        cp_wb(1, 1).start()
        cp_mem().start()

        lane = jax.lax.broadcasted_iota(jnp.int32, (8, 128), 1)

        last = 32 * (lane & 3) + (lane & 28) + (lane >> 5)
        tile = lambda j: pl.ds(j * 128, 128)

        def exchange(t):
            for b in (1, 2, 4):
                t = [jnp.where((lane & (4 * b)) != 0, t[j ^ b], t[j]) for j in range(8)]
            return t

        def permute_q(grp, n):
            for r in range(n):
                t = exchange([grp[r, :, tile(j)] for j in range(8)])
                for j in range(8):
                    grp[r, :, tile(j)] = t[j]
            for j in range(8):
                for r in range(n):
                    grp[r, :, tile(j)] = jnp.take_along_axis(grp[r, :, tile(j)], last ^ (4 * j), axis=1)

        def permute_kv(grp, r, pre, gate):
            t = [gate(grp[r, :, tile(j)]) for j in range(8)]
            if pre:
                t = t[:1] + [jnp.take_along_axis(t[j], lane ^ (4 * j), axis=1) for j in range(1, 8)]
            t = [jnp.take_along_axis(u, last ^ (4 * j), axis=1) for j, u in enumerate(exchange(t))]
            for j in range(8):
                grp[r, :, tile(j)] = t[j]
            return t

        def split_pair(ref, a, b):
            ref[a], ref[b] = _split(ref[a], ref[b])

        for c in range(_QCH):
            cp_wq(c).wait()
            permute_q(wb0.at[pl.ds(c * (RG // _QCH), RG // _QCH)], RG // _QCH)

        def start_pair(hp):
            for cp in cp_pair(hp):
                cp.start()
            cp_xa(hp).start()

        def proj_body(m, i, carry):
            if m == 0:
                pl.when(i + 2 < NB)(lambda: cp_xb(i + 2).start())
                pl.when(i + 2 < NB)(lambda: cp_wb(1, i + 2).start())
                pl.when(i + 2 >= NB)(lambda: cp_wb(2, i + 2 - NB).start())
                pl.when(i < NB - 2)(lambda: cp_woa(i).start())
                pl.when(i >= NB - 2)(lambda: start_pair(i - (NB - 2)))
                cp_xb(i).wait()
            elif m == 1:
                pl.when(i + 2 < NB)(lambda: cp_wb(2, i + 2).start())
                start_pair(i + 2)
            else:
                pl.when(i + 2 < NB)(lambda: start_pair(NB + i + 2))
                pl.when(i >= NB - 2)(lambda: cp_woa(i).start())

                @pl.when(i == NB - 2)
                def _():
                    for cp in cp_wob():
                        cp.start()
            if m < 2:
                cp_wb(m + 1, i).wait()
                nxt = wb[m + 1].at[_rows(i, GPI)]
            if m > 0:
                for cp in cp_pair((m - 1) * NB + i):
                    cp.wait()
                pair = wa.at[_rows((m - 1) * NB + i, 2)]

            dst = qkv.at[m, :, pl.ds(pl.multiple_of(PAD + i * TB, 8), TB), :]
            never = (i + lane) < 0
            gate = lambda u: u
            for j in range(8):
                done = []
                if m < 2:
                    for g in range(j * GPI // 8, (j + 1) * GPI // 8):
                        done += permute_kv(nxt, g, m == 1, gate)
                if m > 0:
                    for g in range(j * RG // 8, (j + 1) * RG // 8):
                        for c in range(3):
                            a, b = _split(gate(pair[0, g, :, tile(c)]), pair[1, g, :, tile(c)])
                            pair[0, g, :, tile(c)], pair[1, g, :, tile(c)] = a, b
                            done += [a, b]
                x = _tie(never, functools.reduce(jnp.bitwise_or, done), xb[_rows(i, TB // 2), :], _TIE_R, _TIE_C)
                r = jnp.dot(_bf16(x), _bf16(wb[m][:, :, tile(j)].reshape(DM // 2, 128)),
                            preferred_element_type=jnp.float32)
                dst[j] = r
                gate = functools.partial(jnp.where, never, pltpu.bitcast(r[0:8], jnp.uint32))
            return carry

        for m in range(3):
            jax.lax.fori_loop(0, NB, functools.partial(proj_body, m), 0)

        pltpu.make_async_copy(woa_h, woa, s_bg.at[0]).wait()
        pltpu.make_async_copy(xa_h, xa, s_bg.at[1]).wait()
        for cp in cp_wob():
            cp.wait()
        cp_mem().wait()
        for dp in range(16):
            for r in range(2):
                split_pair(wob, 4 * dp + r, 4 * dp + 2 + r)
        for m in (1, 2):
            for j in range(8):
                qkv[m, j, 0:PAD, :] = jnp.broadcast_to(qkv[m, j, PAD:PAD + 1, :], (PAD, 128))
        hbuf[0:M, :] = memv[...].astype(jnp.float32)

        row = jax.lax.broadcasted_iota(jnp.int32, (L, 128), 0)
        col = jax.lax.broadcasted_iota(jnp.int32, (L, 128), 1)
        sub = jax.lax.broadcasted_iota(jnp.int32, (8, 128), 0)

        def window_pieces(s, never):
            near = qkv.at[:, :, pl.ds(pl.multiple_of(s * SEG, SEG), PAD + SEG), :]
            st = {}

            def gate(a, tok):
                return jnp.where(never, tok, a)

            def win(m, j, g, w):
                return near[m, j, pl.ds(PAD + g * 8 - DIL * w, 8), :]

            def qk(g, half, tok):
                accs = st.setdefault(("acc", g), [None] * W)
                for j in range(4 * half, 4 * half + 4):
                    qj = gate(win(0, j, g, 0), tok)
                    for w in range(W):
                        p = qj * win(1, j, g, w)
                        accs[w] = p if accs[w] is None else accs[w] + p
                if half == 0:
                    return functools.reduce(jnp.add, accs)
                else:
                    lg = []
                    for w in range(W):
                        a = accs[w]
                        a = a + pltpu.roll(a, 64, 1)
                        a = a + pltpu.roll(a, 32, 1)
                        a = a * scale_b
                        if g * 8 < DIL * w:
                            a = jnp.where(s * SEG + g * 8 + sub >= DIL * w, a, _MASKED)
                        lg.append(a)
                    top = functools.reduce(jnp.maximum, lg)
                    es = [jnp.exp(a - top) for a in lg]
                    st["e", g] = es
                    st["inv", g] = 1.0 / functools.reduce(jnp.add, es)
                    return st["inv", g]

            def pv(g, half, tok):
                inv = gate(st["inv", g], tok)
                ps = [e * inv for e in st["e", g]]
                done = []
                for j in range(4 * half, 4 * half + 4):
                    st["o", g, j] = functools.reduce(jnp.add, [ps[w] * win(2, j, g, w) for w in range(W)])
                    done.append(st["o", g, j])
                    if g % 2 == 1:
                        both = jnp.concatenate([st.pop(("o", g - 1, j)), st.pop(("o", g, j))], axis=0)
                        ob[(g // 2) * 8:(g // 2) * 8 + 8, j * 128:(j + 1) * 128] = _words(both)
                return functools.reduce(jnp.add, done)

            return [functools.partial(fn, g, half)
                    for g in range(SEG // 8) for fn, half in ((qk, 0), (qk, 1), (pv, 0), (pv, 1))]

        def seg_body(s, carry):
            hbuf[M:L, :] = _bf16(xa[_rows(s, SEG // 2), :]).astype(jnp.float32)
            allowed = (row < M) | (row >= col)
            real = col < L
            zpad = jnp.zeros((128 - L, DH), jnp.float32)
            out = outs.at[_rows(s, SEG // 2)]
            never = (s + sub) < 0
            pieces = window_pieces(s, never)
            qs, ks, vs, es, ls = {}, {}, {}, {}, {}

            def project_in(h, done):
                x = hbuf[...] if done is None else _tie(never, done, hbuf[...])
                r = jnp.dot(x, _bf16(wa[h].reshape(DM // 2, 3 * DH)), preferred_element_type=jnp.float32)
                qs[h] = r[:, 0:DH]
                ks[h] = jnp.concatenate([r[:, DH:2 * DH], zpad], axis=0).astype(jnp.bfloat16)
                vs[h] = jnp.concatenate([r[:, 2 * DH:3 * DH], zpad], axis=0).astype(jnp.bfloat16)
                return r[0:8, 0:DH]

            def scores(h):
                sc = jax.lax.dot_general(qs.pop(h), ks.pop(h), _NT, preferred_element_type=jnp.float32) * scale_a
                sc = jnp.where(allowed, sc, _MASKED)
                sc = jnp.where(real, sc, -jnp.inf)
                e = jnp.exp(sc - jnp.max(sc, axis=1, keepdims=True))
                es[h] = e
                ls[h] = 1.0 / jnp.sum(e, axis=1, keepdims=True)

            def values(h):
                obuf[:, h * DH:(h + 1) * DH] = jnp.dot(
                    es.pop(h), vs.pop(h), preferred_element_type=jnp.float32) * ls.pop(h)

            def project_out(h):
                r = jnp.dot(obuf[:, h * DH:(h + WG) * DH], _bf16(woa[h * DH // 2:(h + WG) * DH // 2, :]),
                            preferred_element_type=jnp.float32)
                if h == 0:
                    acc[...] = r
                elif h + WG < H:
                    acc[...] += r
                else:
                    r = r + acc[...]
                    hbuf[0:M, :] = r[0:M]
                    out[:, 0:DM] = _words(r[M:L])

            def window_out(j):
                r = jnp.dot(_bf16(ob[...]), _bf16(wob[:, :, j * 128:(j + 1) * 128].reshape(DM // 2, 128)),
                            preferred_element_type=jnp.float32)
                out[:, DM + j * 128:DM + (j + 1) * 128] = _words(r)

            nxt = 0
            done = {}
            for h in range(H):
                tok = project_in(h, done.pop(h, None))
                if pieces:
                    done[h + _TIE] = pieces.pop(0)(tok)
                if h >= 1:
                    scores(h - 1)
                if h >= 2:
                    values(h - 2)
                if h >= _LAG and (h - _LAG) % WG == 0:
                    project_out(nxt)
                    nxt += WG
            for j in range(0, 4):
                window_out(j)
            scores(H - 1)
            values(H - 2)
            while nxt < H - 2 * WG:
                project_out(nxt)
                nxt += WG
            for j in range(4, 8):
                window_out(j)
            values(H - 1)
            project_out(H - 2 * WG)
            project_out(H - WG)
            cp_out(s).start()
            return carry

        jax.lax.fori_loop(0, S // SEG, seg_body, 0)
        pltpu.make_async_copy(outs, out_h, s_out.at[0]).wait()

    f32, u32 = jnp.float32, jnp.uint32
    scratch = [
        pltpu.VMEM((S // 2, DM), u32),
        pltpu.VMEM((M, DM), jnp.bfloat16),
        pltpu.VMEM((H, RG, 8, 3 * DH), u32),
        pltpu.VMEM((H * DH // 2, DM), u32),
        pltpu.VMEM((S // 2, DM), u32),
        *[pltpu.VMEM((RG, 8, DM), u32)] * 3,
        pltpu.VMEM((RG, 8, DM), u32),
        pltpu.VMEM((3, 8, PAD + S, 128), f32),
        pltpu.VMEM((SEG // 2, DM), u32),
        pltpu.VMEM((S // 2, 2 * DM), u32),
        pltpu.VMEM((L, DM), f32),
        pltpu.VMEM((L, H * DH), f32),
        pltpu.VMEM((L, DM), f32),
        pltpu.SemaphoreType.DMA((_QCH,)),
        pltpu.SemaphoreType.DMA((2 * NB,)),
        pltpu.SemaphoreType.DMA((NB,)),
        pltpu.SemaphoreType.DMA((NPAIR,)),
        pltpu.SemaphoreType.DMA((4,)),
        pltpu.SemaphoreType.DMA((1,)),
    ]
    return kernel, scratch


def pallas_concat_heads__memory_aug_recurrent_mem_tr__sliding_local_dilated__prompt_kernel(
    A_x, A_mem0, A_Wq, A_Wk, A_Wv, A_Wo, A_seg_len, B_x, B_wqkv, B_wo,
):
    B, S, DM = A_x.shape
    H, DH = A_Wq.shape[1], A_Wq.shape[2]
    M = A_mem0.shape[1]
    assert B == 1 and B_x.shape == (1, S, DM)
    kernel, scratch = _make_kernel(S, DM, H, DH, M, int(A_seg_len))
    heads = lambda w: w.reshape(DM // 16, 2, 8, H, DH)
    out = pl.pallas_call(
        kernel,
        out_shape=jax.ShapeDtypeStruct((S, 2 * DM), jnp.bfloat16),
        in_specs=[pl.BlockSpec(memory_space=pl.ANY)] * 9,
        out_specs=pl.BlockSpec(memory_space=pl.ANY),
        scratch_shapes=scratch,
        compiler_params=pltpu.CompilerParams(vmem_limit_bytes=110 * 1024 * 1024),
    )(
        A_x.reshape(S, DM), A_mem0.reshape(M, DM), heads(A_Wq), heads(A_Wk), heads(A_Wv),
        A_Wo.reshape(H * DH, DM), B_x.reshape(S, DM), B_wqkv.reshape(DM // 16, 16, 3 * DM),
        B_wo.reshape(_HB // 16, 2, 8, DM // _HB, DM),
    )
    return out.reshape(1, S, 2 * DM)
```

```python
import functools

import jax
import jax.numpy as jnp
import jax.experimental.pallas as pl
import jax.experimental.pallas.tpu as pltpu

_NT = (((1,), (1,)), ((), ()))
_MASKED = -1000000000.0

_HB, _W, _DIL = 32, 8, 2
_PAD = 16
_TB = 256
_WG = 4
_LAG = 19
_TIE = 2
_TAIL = 8
_UNROLL = 4
_TIE_R, _TIE_C = 64, 512
_QCH = 4


def _split(a, b):
    u = jnp.concatenate([a, b], axis=0)
    lo = pltpu.bitcast(u << 16, jnp.float32).astype(jnp.bfloat16)
    hi = pltpu.bitcast(u & jnp.uint32(0xFFFF0000), jnp.float32).astype(jnp.bfloat16)
    return pltpu.bitcast(lo, jnp.uint32), pltpu.bitcast(hi, jnp.uint32)


def _bf16(u):
    return pltpu.bitcast(u, jnp.bfloat16)


def _words(x):
    return pltpu.bitcast(x.astype(jnp.bfloat16), jnp.uint32)


def _tie(never, tok, x, r=0, c=0):
    cat = lambda parts, axis: jnp.concatenate([p for p in parts if p.size], axis=axis)
    mid = cat([x[r:r + 8, :c], jnp.where(never, tok, x[r:r + 8, c:c + 128]), x[r:r + 8, c + 128:]], 1)
    return cat([x[:r], mid, x[r + 8:]], 0)


def _rows(i, n):
    return pl.ds(i * n, n) if isinstance(i, int) else pl.ds(pl.multiple_of(i * n, n), n)


def _make_kernel(S, DM, H, DH, M, SEG):
    L = M + SEG
    PAD, W, DIL, TB, WG = _PAD, _W, _DIL, _TB, _WG
    NB = S // TB
    NPAIR = H // 2
    RG = DM // 16
    GPI = RG // NB
    assert DM == 1024 and DH == 128 and DM // _HB == 32 and NPAIR == 2 * NB and PAD >= DIL * (W - 1)
    scale_a = DH ** -0.5
    scale_b = (DM // _HB) ** -0.5

    def kernel(xa_hbm, mem_hbm, wq_hbm, wk_hbm, wv_hbm, woa_hbm, xb_hbm, wb_hbm, wob_hbm,
               out_hbm,
               xa, memv, wa, woa, xb, wb0, wb1, wb2, wob, qkv, ob, outs, hbuf, obuf, acc,
               s_wq, s_wb, s_xb, s_pair, s_bg, s_out):
        u32 = lambda r: r.bitcast(jnp.uint32)
        xa_h, woa_h, xb_h, wb_h, wob_h, out_h = (
            u32(xa_hbm), u32(woa_hbm), u32(xb_hbm), u32(wb_hbm), u32(wob_hbm), u32(out_hbm))
        wa_h = [u32(wq_hbm), u32(wk_hbm), u32(wv_hbm)]
        wb = [wb0, wb1, wb2]

        def cp_wq(c):
            n = RG // _QCH
            return pltpu.make_async_copy(wb_h.at[pl.ds(c * n, n), :, pl.ds(0, DM)], wb0.at[pl.ds(c * n, n)], s_wq.at[c])

        def cp_wb(m, c):
            return pltpu.make_async_copy(wb_h.at[_rows(c, GPI), :, pl.ds(m * DM, DM)], wb[m].at[_rows(c, GPI)],
                                         s_wb.at[(m - 1) * NB + c])

        def cp_xb(c):
            return pltpu.make_async_copy(xb_h.at[_rows(c, TB // 2)], xb.at[_rows(c, TB // 2)], s_xb.at[c])

        def cp_pair(hp):
            return [pltpu.make_async_copy(wa_h[m].at[:, e, :, hp, :],
                                          wa.at[2 * hp + e, :, :, pl.ds(m * DH, DH)], s_pair.at[hp])
                    for m in range(3) for e in range(2)]

        def cp_woa(c):
            n = H * DH // 16
            return pltpu.make_async_copy(woa_h.at[_rows(c, n)], woa.at[_rows(c, n)], s_bg.at[0])

        def cp_xa(c):
            n = S // 2 // NPAIR
            return pltpu.make_async_copy(xa_h.at[_rows(c, n)], xa.at[_rows(c, n)], s_bg.at[1])

        def cp_wob():
            return [pltpu.make_async_copy(wob_h.at[:, e, :, dp, :], wob.at[pl.ds(2 * (2 * dp + e), 2)], s_bg.at[2])
                    for dp in range(16) for e in range(2)]

        def cp_mem():
            return pltpu.make_async_copy(mem_hbm, memv, s_bg.at[3])

        def cp_out(s):
            n = _UNROLL * SEG // 2
            return pltpu.make_async_copy(outs.at[_rows(s, n)], out_h.at[_rows(s, n)], s_out.at[0])

        cp_xb(0).start()
        for c in range(_QCH):
            cp_wq(c).start()
        cp_wb(1, 0).start()
        cp_xb(1).start()
        cp_wb(1, 1).start()
        cp_mem().start()

        lane = jax.lax.broadcasted_iota(jnp.int32, (8, 128), 1)

        last = 32 * (lane & 3) + (lane & 28) + (lane >> 5)
        tile = lambda j: pl.ds(j * 128, 128)

        def exchange(t):
            for b in (1, 2, 4):
                t = [jnp.where((lane & (4 * b)) != 0, t[j ^ b], t[j]) for j in range(8)]
            return t

        def permute_q(grp, n):
            for r in range(n):
                t = exchange([grp[r, :, tile(j)] for j in range(8)])
                for j in range(8):
                    grp[r, :, tile(j)] = t[j]
            for j in range(8):
                for r in range(n):
                    grp[r, :, tile(j)] = jnp.take_along_axis(grp[r, :, tile(j)], last ^ (4 * j), axis=1)

        def permute_kv(grp, r, pre, gate):
            t = [gate(grp[r, :, tile(j)]) for j in range(8)]
            if pre:
                t = t[:1] + [jnp.take_along_axis(t[j], lane ^ (4 * j), axis=1) for j in range(1, 8)]
            t = [jnp.take_along_axis(u, last ^ (4 * j), axis=1) for j, u in enumerate(exchange(t))]
            for j in range(8):
                grp[r, :, tile(j)] = t[j]
            return t

        def split_pair(ref, a, b):
            ref[a], ref[b] = _split(ref[a], ref[b])

        for c in range(_QCH):
            cp_wq(c).wait()
            permute_q(wb0.at[pl.ds(c * (RG // _QCH), RG // _QCH)], RG // _QCH)

        def start_pair(hp):
            for cp in cp_pair(hp):
                cp.start()
            cp_xa(hp).start()

        def proj_body(m, i, carry):
            if m == 0:
                pl.when(i + 2 < NB)(lambda: cp_xb(i + 2).start())
                pl.when(i + 2 < NB)(lambda: cp_wb(1, i + 2).start())
                pl.when(i + 2 >= NB)(lambda: cp_wb(2, i + 2 - NB).start())
                pl.when(i < NB - 2)(lambda: cp_woa(i).start())
                pl.when(i >= NB - 2)(lambda: start_pair(i - (NB - 2)))
                cp_xb(i).wait()
            elif m == 1:
                pl.when(i + 2 < NB)(lambda: cp_wb(2, i + 2).start())
                start_pair(i + 2)
            else:
                pl.when(i + 2 < NB)(lambda: start_pair(NB + i + 2))
                pl.when(i >= NB - 2)(lambda: cp_woa(i).start())

                @pl.when(i == NB - 2)
                def _():
                    for cp in cp_wob():
                        cp.start()
            if m < 2:
                cp_wb(m + 1, i).wait()
                nxt = wb[m + 1].at[_rows(i, GPI)]
            if m > 0:
                for cp in cp_pair((m - 1) * NB + i):
                    cp.wait()
                pair = wa.at[_rows((m - 1) * NB + i, 2)]

            dst = qkv.at[m, :, pl.ds(pl.multiple_of(PAD + i * TB, 8), TB), :]
            never = (i + lane) < 0
            gate = lambda u: u
            for j in range(8):
                done = []
                if m < 2:
                    for g in range(j * GPI // 8, (j + 1) * GPI // 8):
                        done += permute_kv(nxt, g, m == 1, gate)
                if m > 0:
                    for g in range(j * RG // 8, (j + 1) * RG // 8):
                        for c in range(3):
                            a, b = _split(gate(pair[0, g, :, tile(c)]), pair[1, g, :, tile(c)])
                            pair[0, g, :, tile(c)], pair[1, g, :, tile(c)] = a, b
                            done += [a, b]
                x = _tie(never, functools.reduce(jnp.bitwise_or, done), xb[_rows(i, TB // 2), :], _TIE_R, _TIE_C)
                r = jnp.dot(_bf16(x), _bf16(wb[m][:, :, tile(j)].reshape(DM // 2, 128)),
                            preferred_element_type=jnp.float32)
                dst[j] = r
                gate = functools.partial(jnp.where, never, pltpu.bitcast(r[0:8], jnp.uint32))
            return carry

        for m in range(3):
            jax.lax.fori_loop(0, NB, functools.partial(proj_body, m), 0)

        pltpu.make_async_copy(woa_h, woa, s_bg.at[0]).wait()
        pltpu.make_async_copy(xa_h, xa, s_bg.at[1]).wait()
        for cp in cp_wob():
            cp.wait()
        cp_mem().wait()
        for dp in range(16):
            for r in range(2):
                split_pair(wob, 4 * dp + r, 4 * dp + 2 + r)
        for m in (1, 2):
            for j in range(8):
                qkv[m, j, 0:PAD, :] = jnp.broadcast_to(qkv[m, j, PAD:PAD + 1, :], (PAD, 128))
        hbuf[0:M, :] = memv[...].astype(jnp.float32)

        row = jax.lax.broadcasted_iota(jnp.int32, (L, 128), 0)
        col = jax.lax.broadcasted_iota(jnp.int32, (L, 128), 1)
        sub = jax.lax.broadcasted_iota(jnp.int32, (8, 128), 0)

        def window_pieces(s, never):
            near = qkv.at[:, :, pl.ds(pl.multiple_of(s * SEG, SEG), PAD + SEG), :]
            st = {}

            def gate(a, tok):
                return jnp.where(never, tok, a)

            def win(m, j, g, w):
                return near[m, j, pl.ds(PAD + g * 8 - DIL * w, 8), :]

            def qk(g, half, tok):
                accs = st.setdefault(("acc", g), [None] * W)
                for j in range(4 * half, 4 * half + 4):
                    qj = gate(win(0, j, g, 0), tok)
                    for w in range(W):
                        p = qj * win(1, j, g, w)
                        accs[w] = p if accs[w] is None else accs[w] + p
                if half == 0:
                    return functools.reduce(jnp.add, accs)
                else:
                    lg = []
                    for w in range(W):
                        a = accs[w]
                        a = a + pltpu.roll(a, 64, 1)
                        a = a + pltpu.roll(a, 32, 1)
                        a = a * scale_b
                        if g * 8 < DIL * w:
                            a = jnp.where(s * SEG + g * 8 + sub >= DIL * w, a, _MASKED)
                        lg.append(a)
                    top = functools.reduce(jnp.maximum, lg)
                    es = [jnp.exp(a - top) for a in lg]
                    st["e", g] = es
                    st["inv", g] = 1.0 / functools.reduce(jnp.add, es)
                    return st["inv", g]

            def pv(g, half, tok):
                inv = gate(st["inv", g], tok)
                ps = [e * inv for e in st["e", g]]
                done = []
                for j in range(4 * half, 4 * half + 4):
                    st["o", g, j] = functools.reduce(jnp.add, [ps[w] * win(2, j, g, w) for w in range(W)])
                    done.append(st["o", g, j])
                    if g % 2 == 1:
                        both = jnp.concatenate([st.pop(("o", g - 1, j)), st.pop(("o", g, j))], axis=0)
                        ob[(g // 2) * 8:(g // 2) * 8 + 8, j * 128:(j + 1) * 128] = _words(both)
                return functools.reduce(jnp.add, done)

            return [functools.partial(fn, g, half)
                    for g in range(SEG // 8) for fn, half in ((qk, 0), (qk, 1), (pv, 0), (pv, 1))]

        def step(s):
            hbuf[M:L, :] = _bf16(xa[_rows(s, SEG // 2), :]).astype(jnp.float32)
            allowed = (row < M) | (row >= col)
            real = col < L
            zpad = jnp.zeros((128 - L, DH), jnp.float32)
            out = outs.at[_rows(s, SEG // 2)]
            never = (s + sub) < 0
            pieces = window_pieces(s, never)
            qs, ks, vs, es, ls = {}, {}, {}, {}, {}

            def project_in(h, done):
                x = hbuf[...] if done is None else _tie(never, done, hbuf[...])
                r = jnp.dot(x, _bf16(wa[h].reshape(DM // 2, 3 * DH)), preferred_element_type=jnp.float32)
                qs[h] = r[:, 0:DH]
                ks[h] = jnp.concatenate([r[:, DH:2 * DH], zpad], axis=0).astype(jnp.bfloat16)
                vs[h] = jnp.concatenate([r[:, 2 * DH:3 * DH], zpad], axis=0).astype(jnp.bfloat16)
                return r[0:8, 0:DH]

            def scores(h):
                sc = jax.lax.dot_general(qs.pop(h), ks.pop(h), _NT, preferred_element_type=jnp.float32) * scale_a
                sc = jnp.where(allowed, sc, _MASKED)
                sc = jnp.where(real, sc, -jnp.inf)
                e = jnp.exp(sc - jnp.max(sc, axis=1, keepdims=True))
                es[h] = e
                ls[h] = 1.0 / jnp.sum(e, axis=1, keepdims=True)

            def values(h):
                obuf[:, h * DH:(h + 1) * DH] = jnp.dot(
                    es.pop(h), vs.pop(h), preferred_element_type=jnp.float32) * ls.pop(h)

            def project_out(h):
                r = jnp.dot(obuf[:, h * DH:(h + WG) * DH], _bf16(woa[h * DH // 2:(h + WG) * DH // 2, :]),
                            preferred_element_type=jnp.float32)
                if h == 0:
                    acc[...] = r
                elif h + WG < H:
                    acc[...] += r
                else:
                    r = r + acc[...]
                    hbuf[0:M, :] = r[0:M]
                    out[:, 0:DM] = _words(r[M:L])

            def window_out(j):
                r = jnp.dot(_bf16(ob[...]), _bf16(wob[:, :, j * 128:(j + 1) * 128].reshape(DM // 2, 128)),
                            preferred_element_type=jnp.float32)
                out[:, DM + j * 128:DM + (j + 1) * 128] = _words(r)

            nxt = 0
            done = {}
            for h in range(H):
                tok = project_in(h, done.pop(h, None))
                if pieces:
                    done[h + _TIE] = pieces.pop(0)(tok)
                if h >= 1:
                    scores(h - 1)
                if h >= 2:
                    values(h - 2)
                if h >= _LAG and (h - _LAG) % WG == 0:
                    project_out(nxt)
                    nxt += WG
            if _TAIL == 0:
                for j in range(0, 4):
                    window_out(j)
                scores(H - 1)
                values(H - 2)
                while nxt < H - 2 * WG:
                    project_out(nxt)
                    nxt += WG
                for j in range(4, 8):
                    window_out(j)
                values(H - 1)
                project_out(H - 2 * WG)
                project_out(H - WG)
            else:
                while nxt < H - 3 * WG:
                    project_out(nxt)
                    nxt += WG
                scores(H - 1)
                values(H - 2)
                project_out(H - 3 * WG)
                for j in range(0, 8 - _TAIL):
                    window_out(j)
                values(H - 1)
                project_out(H - 2 * WG)
                project_out(H - WG)
                for j in range(8 - _TAIL, 8):
                    window_out(j)

        def seg_body(i, carry):
            for u in range(_UNROLL):
                step(i * _UNROLL + u)
            cp_out(i).start()
            return carry

        jax.lax.fori_loop(0, S // SEG // _UNROLL, seg_body, 0)
        pltpu.make_async_copy(outs, out_h, s_out.at[0]).wait()

    f32, u32 = jnp.float32, jnp.uint32
    scratch = [
        pltpu.VMEM((S // 2, DM), u32),
        pltpu.VMEM((M, DM), jnp.bfloat16),
        pltpu.VMEM((H, RG, 8, 3 * DH), u32),
        pltpu.VMEM((H * DH // 2, DM), u32),
        pltpu.VMEM((S // 2, DM), u32),
        *[pltpu.VMEM((RG, 8, DM), u32)] * 3,
        pltpu.VMEM((RG, 8, DM), u32),
        pltpu.VMEM((3, 8, PAD + S, 128), f32),
        pltpu.VMEM((SEG // 2, DM), u32),
        pltpu.VMEM((S // 2, 2 * DM), u32),
        pltpu.VMEM((L, DM), f32),
        pltpu.VMEM((L, H * DH), f32),
        pltpu.VMEM((L, DM), f32),
        pltpu.SemaphoreType.DMA((_QCH,)),
        pltpu.SemaphoreType.DMA((2 * NB,)),
        pltpu.SemaphoreType.DMA((NB,)),
        pltpu.SemaphoreType.DMA((NPAIR,)),
        pltpu.SemaphoreType.DMA((4,)),
        pltpu.SemaphoreType.DMA((1,)),
    ]
    return kernel, scratch


def pallas_concat_heads__memory_aug_recurrent_mem_tr__sliding_local_dilated__prompt_kernel(
    A_x, A_mem0, A_Wq, A_Wk, A_Wv, A_Wo, A_seg_len, B_x, B_wqkv, B_wo,
):
    B, S, DM = A_x.shape
    H, DH = A_Wq.shape[1], A_Wq.shape[2]
    M = A_mem0.shape[1]
    assert B == 1 and B_x.shape == (1, S, DM)
    kernel, scratch = _make_kernel(S, DM, H, DH, M, int(A_seg_len))
    heads = lambda w: w.reshape(DM // 16, 2, 8, H, DH)
    out = pl.pallas_call(
        kernel,
        out_shape=jax.ShapeDtypeStruct((S, 2 * DM), jnp.bfloat16),
        in_specs=[pl.BlockSpec(memory_space=pl.ANY)] * 9,
        out_specs=pl.BlockSpec(memory_space=pl.ANY),
        scratch_shapes=scratch,
        compiler_params=pltpu.CompilerParams(vmem_limit_bytes=110 * 1024 * 1024),
    )(
        A_x.reshape(S, DM), A_mem0.reshape(M, DM), heads(A_Wq), heads(A_Wk), heads(A_Wv),
        A_Wo.reshape(H * DH, DM), B_x.reshape(S, DM), B_wqkv.reshape(DM // 16, 16, 3 * DM),
        B_wo.reshape(_HB // 16, 2, 8, DM // _HB, DM),
    )
    return out.reshape(1, S, 2 * DM)
```

```python
import functools

import jax
import jax.numpy as jnp
import jax.experimental.pallas as pl
import jax.experimental.pallas.tpu as pltpu

_NT = (((1,), (1,)), ((), ()))
_MASKED = -1000000000.0

_HB, _W, _DIL = 32, 8, 2
_PAD = 16
_TB = 512
_TS = 256
_WG = 4
_LAG = 19
_TIE = 2
_TAIL = 8
_UNROLL = 4
_TIES = ((32, 0), (96, 0), (32, 512), (96, 512))


def _split(a, b):
    u = jnp.concatenate([a, b], axis=0)
    lo = pltpu.bitcast(u << 16, jnp.float32).astype(jnp.bfloat16)
    hi = pltpu.bitcast(u & jnp.uint32(0xFFFF0000), jnp.float32).astype(jnp.bfloat16)
    return pltpu.bitcast(lo, jnp.uint32), pltpu.bitcast(hi, jnp.uint32)


def _bf16(u):
    return pltpu.bitcast(u, jnp.bfloat16)


def _words(x):
    return pltpu.bitcast(x.astype(jnp.bfloat16), jnp.uint32)


def _tie(never, tok, x, r=0, c=0):
    cat = lambda parts, axis: jnp.concatenate([p for p in parts if p.size], axis=axis)
    mid = cat([x[r:r + 8, :c], jnp.where(never, tok, x[r:r + 8, c:c + 128]), x[r:r + 8, c + 128:]], 1)
    return cat([x[:r], mid, x[r + 8:]], 0)


def tile(j):
    return pl.ds(j * 128, 128)


def _rows(i, n):
    return pl.ds(i * n, n) if isinstance(i, int) else pl.ds(pl.multiple_of(i * n, n), n)


def _make_kernel(S, DM, H, DH, M, SEG):
    L = M + SEG
    PAD, W, DIL, TB, TS, WG = _PAD, _W, _DIL, _TB, _TS, _WG
    NB = S // TB
    NPAIR = H // 2
    UN = _UNROLL
    NSTEP = S // SEG // UN
    RG = DM // 16
    KT = DM // 128
    PPI = NPAIR // (2 * NB)
    DPI = 16 // NB
    GPI = RG // NB
    assert DM == 1024 and DH == 128 and DM // _HB == 32 and NPAIR == 2 * NB * PPI and PAD >= DIL * (W - 1)
    scale_a = DH ** -0.5
    scale_b = (DM // _HB) ** -0.5

    def kernel(xa_hbm, mem_hbm, wq_hbm, wk_hbm, wv_hbm, woa_hbm, xb_hbm, wb_hbm, wob_hbm,
               out_hbm,
               xa, memv, wa, woa, xb, wb0, wb1, wb2, wob, qkv, ob, outs, hbuf, obuf, acc,
               s_wq, s_wb, s_xb, s_pair, s_wob, s_xa, s_misc, s_out):
        u32 = lambda r: r.bitcast(jnp.uint32)
        xa_h, woa_h, xb_h, wb_h, wob_h, out_h = (
            u32(xa_hbm), u32(woa_hbm), u32(xb_hbm), u32(wb_hbm), u32(wob_hbm), u32(out_hbm))
        wa_h = [u32(wq_hbm), u32(wk_hbm), u32(wv_hbm)]
        wb = [wb0, wb1, wb2]

        def cp_first(c):
            n = RG // KT
            return [pltpu.make_async_copy(wb_h.at[pl.ds(c * n, n), :, pl.ds(0, DM)], wb0.at[pl.ds(c * n, n)], s_wq.at[c]),
                    pltpu.make_async_copy(xb_h.at[pl.ds(0, TB // 2), tile(c)], xb.at[pl.ds(0, TB // 2), tile(c)], s_wq.at[c])]

        def cp_wb(m, c):
            return pltpu.make_async_copy(wb_h.at[_rows(c, GPI), :, pl.ds(m * DM, DM)], wb[m].at[_rows(c, GPI)],
                                         s_wb.at[(m - 1) * NB + c])

        def cp_xb(c):
            return pltpu.make_async_copy(xb_h.at[_rows(c, TB // 2)], xb.at[_rows(c, TB // 2)], s_xb.at[c])

        def cp_pair(hp):
            return [pltpu.make_async_copy(wa_h[m].at[:, :, :, hp, :], wa.at[hp, :, :, :, tile(m)], s_pair.at[hp // PPI])
                    for m in range(3)]

        def cp_wob(dp):
            return pltpu.make_async_copy(wob_h.at[:, :, :, dp, :], wob.at[dp], s_wob.at[dp // DPI])

        def cp_woa():
            return pltpu.make_async_copy(woa_h, woa, s_misc.at[0])

        def cp_xa(i):
            return pltpu.make_async_copy(xa_h.at[_rows(i, UN * SEG // 2)], xa.at[_rows(i, UN * SEG // 2)], s_xa.at[i])

        def cp_mem():
            return pltpu.make_async_copy(mem_hbm, memv, s_misc.at[1])

        def cp_out(s):
            n = UN * SEG // 2
            return pltpu.make_async_copy(outs.at[_rows(s, n)], out_h.at[_rows(s, n)], s_out.at[0])

        def start_pairs(q):
            for u in range(PPI):
                for cp in cp_pair(q * PPI + u):
                    cp.start()

        for c in range(KT):
            for cp in cp_first(c):
                cp.start()
        cp_wb(1, 0).start()
        for i in range(1, NB):
            cp_xb(i).start()
            cp_wb(1, i).start()
        for i in range(NB):
            cp_wb(2, i).start()
            start_pairs(i)

        def wait_filled(buf, sem):
            pltpu.make_async_copy(buf, buf, sem).wait()

        lane = jax.lax.broadcasted_iota(jnp.int32, (8, 128), 1)

        last = 32 * (lane & 3) + (lane & 28) + (lane >> 5)

        def exchange(t):
            for b in (1, 2, 4):
                t = [jnp.where((lane & (4 * b)) != 0, t[j ^ b], t[j]) for j in range(8)]
            return t

        def permute(grp, r, pre, gate):
            t = [gate(grp[r, :, tile(j)]) for j in range(8)]
            if pre:
                t = t[:1] + [jnp.take_along_axis(t[j], lane ^ (4 * j), axis=1) for j in range(1, 8)]
            t = [jnp.take_along_axis(u, last ^ (4 * j), axis=1) for j, u in enumerate(exchange(t))]
            for j in range(8):
                grp[r, :, tile(j)] = t[j]
            return t

        def split(ref, idx, gate):
            a, b = _split(gate(ref[idx(0)]), ref[idx(1)])
            ref[idx(0)], ref[idx(1)] = a, b
            return [a, b]

        def first_block():
            same = lambda u: u
            n = RG // KT
            dst = qkv.at[0, :, pl.ds(PAD, TB), :]
            for cp in cp_first(0):
                cp.wait()
            for g in range(n):
                permute(wb0, g, False, same)
            for c in range(KT):
                if c + 1 < KT:
                    for cp in cp_first(c + 1):
                        cp.wait()
                    for g in range(n):
                        permute(wb0, (c + 1) * n + g, False, same)
                else:
                    cp_wb(1, 0).wait()
                    for g in range(GPI):
                        permute(wb1, g, False, same)
                x = _bf16(xb[0:TB // 2, tile(c)])
                for j in range(8):
                    r = jnp.dot(x, _bf16(wb0[c * n:(c + 1) * n, :, tile(j)].reshape(64, 128)),
                                preferred_element_type=jnp.float32)
                    dst[j] = r if c == 0 else dst[j] + r

        def proj_body(m, i, carry):
            if m == 0:
                cp_xb(i).wait()
            elif m == 1:
                for u in range(DPI):
                    cp_wob(i * DPI + u).start()
                start_pairs(NB + i)
            else:
                for u in range(NSTEP // NB):
                    cp_xa(i * (NSTEP // NB) + u).start()
            if m < 2:
                cp_wb(m + 1, i).wait()
                nxt = wb[m + 1].at[_rows(i, GPI)]
            else:
                dims = wob.at[_rows(i, DPI)]
                wait_filled(dims, s_wob.at[i])
            if m > 0:
                pairs = wa.at[_rows((m - 1) * NB + i, PPI)]
                wait_filled(pairs, s_pair.at[(m - 1) * NB + i])

            work = []
            if m < 2:
                work.append([functools.partial(permute, nxt, g, m == 1) for g in range(GPI)])
            else:
                work.append([functools.partial(split, dims, lambda e, u=u, r=r, c=c: (u, r, e, slice(None), tile(c)))
                             for u in range(DPI) for r in range(2) for c in range(8)])
            if m > 0:
                work.append([functools.partial(split, pairs, lambda e, u=u, g=g, c=c: (u, g, e, slice(None), tile(c)))
                             for u in range(PPI) for g in range(RG) for c in range(3)])

            dst = qkv.at[m, :, pl.ds(pl.multiple_of(PAD + i * TB, 8), TB), :]
            never = (i + lane) < 0
            gate = lambda u: u
            slots = [(j, t) for j in range(8) for t in range(0, TB, TS)]
            for n, (j, t) in enumerate(slots):
                x = xb[pl.ds(pl.multiple_of(i * (TB // 2) + t // 2, TS // 2), TS // 2), :]
                for a, at in enumerate(_TIES):
                    part, parts = n * len(_TIES) + a, len(slots) * len(_TIES)
                    done = [u for jobs in work
                            for job in jobs[part * len(jobs) // parts:(part + 1) * len(jobs) // parts]
                            for u in job(gate)]
                    if done:
                        x = _tie(never, functools.reduce(jnp.bitwise_or, done), x, *at)
                r = jnp.dot(_bf16(x), _bf16(wb[m][:, :, tile(j)].reshape(DM // 2, 128)),
                            preferred_element_type=jnp.float32)
                dst[j, t:t + TS, :] = r
                gate = functools.partial(jnp.where, never, pltpu.bitcast(r[0:8], jnp.uint32))
            return carry

        first_block()
        for m in range(3):
            if m == 2:
                cp_woa().start()
                cp_mem().start()
            jax.lax.fori_loop(1 if m == 0 else 0, NB, functools.partial(proj_body, m), 0)

        cp_mem().wait()
        cp_woa().wait()
        for m in (1, 2):
            for j in range(8):
                qkv[m, j, 0:PAD, :] = jnp.broadcast_to(qkv[m, j, PAD:PAD + 1, :], (PAD, 128))
        hbuf[0:M, :] = memv[...].astype(jnp.float32)

        row = jax.lax.broadcasted_iota(jnp.int32, (L, 128), 0)
        col = jax.lax.broadcasted_iota(jnp.int32, (L, 128), 1)
        sub = jax.lax.broadcasted_iota(jnp.int32, (8, 128), 0)

        def window_pieces(s, never):
            near = qkv.at[:, :, pl.ds(pl.multiple_of(s * SEG, SEG), PAD + SEG), :]
            st = {}

            def gate(a, tok):
                return jnp.where(never, tok, a)

            def win(m, j, g, w):
                return near[m, j, pl.ds(PAD + g * 8 - DIL * w, 8), :]

            def qk(g, half, tok):
                accs = st.setdefault(("acc", g), [None] * W)
                for j in range(4 * half, 4 * half + 4):
                    qj = gate(win(0, j, g, 0), tok)
                    for w in range(W):
                        p = qj * win(1, j, g, w)
                        accs[w] = p if accs[w] is None else accs[w] + p
                if half == 0:
                    return functools.reduce(jnp.add, accs)
                else:
                    lg = []
                    for w in range(W):
                        a = accs[w]
                        a = a + pltpu.roll(a, 64, 1)
                        a = a + pltpu.roll(a, 32, 1)
                        a = a * scale_b
                        if g * 8 < DIL * w:
                            a = jnp.where(s * SEG + g * 8 + sub >= DIL * w, a, _MASKED)
                        lg.append(a)
                    top = functools.reduce(jnp.maximum, lg)
                    es = [jnp.exp(a - top) for a in lg]
                    st["e", g] = es
                    st["inv", g] = 1.0 / functools.reduce(jnp.add, es)
                    return st["inv", g]

            def pv(g, half, tok):
                inv = gate(st["inv", g], tok)
                ps = [e * inv for e in st["e", g]]
                done = []
                for j in range(4 * half, 4 * half + 4):
                    st["o", g, j] = functools.reduce(jnp.add, [ps[w] * win(2, j, g, w) for w in range(W)])
                    done.append(st["o", g, j])
                    if g % 2 == 1:
                        both = jnp.concatenate([st.pop(("o", g - 1, j)), st.pop(("o", g, j))], axis=0)
                        ob[(g // 2) * 8:(g // 2) * 8 + 8, j * 128:(j + 1) * 128] = _words(both)
                return functools.reduce(jnp.add, done)

            return [functools.partial(fn, g, half)
                    for g in range(SEG // 8) for fn, half in ((qk, 0), (qk, 1), (pv, 0), (pv, 1))]

        def step(s):
            hbuf[M:L, :] = _bf16(xa[_rows(s, SEG // 2), :]).astype(jnp.float32)
            allowed = (row < M) | (row >= col)
            real = col < L
            zpad = jnp.zeros((128 - L, DH), jnp.float32)
            out = outs.at[_rows(s, SEG // 2)]
            never = (s + sub) < 0
            pieces = window_pieces(s, never)
            qs, ks, vs, es, ls = {}, {}, {}, {}, {}

            def project_in(h, done):
                x = hbuf[...] if done is None else _tie(never, done, hbuf[...])
                r = jnp.dot(x, _bf16(wa[h // 2, :, h % 2].reshape(DM // 2, 3 * DH)), preferred_element_type=jnp.float32)
                qs[h] = r[:, 0:DH]
                ks[h] = jnp.concatenate([r[:, DH:2 * DH], zpad], axis=0).astype(jnp.bfloat16)
                vs[h] = jnp.concatenate([r[:, 2 * DH:3 * DH], zpad], axis=0).astype(jnp.bfloat16)
                return r[0:8, 0:DH]

            def scores(h):
                sc = jax.lax.dot_general(qs.pop(h), ks.pop(h), _NT, preferred_element_type=jnp.float32) * scale_a
                sc = jnp.where(allowed, sc, _MASKED)
                sc = jnp.where(real, sc, -jnp.inf)
                e = jnp.exp(sc - jnp.max(sc, axis=1, keepdims=True))
                es[h] = e
                ls[h] = 1.0 / jnp.sum(e, axis=1, keepdims=True)

            def values(h):
                obuf[:, h * DH:(h + 1) * DH] = jnp.dot(
                    es.pop(h), vs.pop(h), preferred_element_type=jnp.float32) * ls.pop(h)

            def project_out(h):
                r = jnp.dot(obuf[:, h * DH:(h + WG) * DH], _bf16(woa[h * DH // 2:(h + WG) * DH // 2, :]),
                            preferred_element_type=jnp.float32)
                if h == 0:
                    acc[...] = r
                elif h + WG < H:
                    acc[...] += r
                else:
                    r = r + acc[...]
                    hbuf[0:M, :] = r[0:M]
                    out[:, 0:DM] = _words(r[M:L])

            def window_out(j):
                w = jnp.concatenate([wob[dp, r, e, :, tile(j)] for dp in range(16) for e in range(2) for r in range(2)], axis=0)
                r = jnp.dot(_bf16(ob[...]), _bf16(w), preferred_element_type=jnp.float32)
                out[:, DM + j * 128:DM + (j + 1) * 128] = _words(r)

            nxt = 0
            done = {}
            for h in range(H):
                tok = project_in(h, done.pop(h, None))
                if pieces:
                    done[h + _TIE] = pieces.pop(0)(tok)
                if h >= 1:
                    scores(h - 1)
                if h >= 2:
                    values(h - 2)
                if h >= _LAG and (h - _LAG) % WG == 0:
                    project_out(nxt)
                    nxt += WG
            if _TAIL == 0:
                for j in range(0, 4):
                    window_out(j)
                scores(H - 1)
                values(H - 2)
                while nxt < H - 2 * WG:
                    project_out(nxt)
                    nxt += WG
                for j in range(4, 8):
                    window_out(j)
                values(H - 1)
                project_out(H - 2 * WG)
                project_out(H - WG)
            else:
                while nxt < H - 3 * WG:
                    project_out(nxt)
                    nxt += WG
                scores(H - 1)
                values(H - 2)
                project_out(H - 3 * WG)
                for j in range(0, 8 - _TAIL):
                    window_out(j)
                values(H - 1)
                project_out(H - 2 * WG)
                project_out(H - WG)
                for j in range(8 - _TAIL, 8):
                    window_out(j)

        def seg_body(i, carry):
            cp_xa(i).wait()
            for u in range(UN):
                step(i * UN + u)
            cp_out(i).start()
            return carry

        jax.lax.fori_loop(0, NSTEP, seg_body, 0)
        pltpu.make_async_copy(outs, out_h, s_out.at[0]).wait()

    f32, u32 = jnp.float32, jnp.uint32
    scratch = [
        pltpu.VMEM((S // 2, DM), u32),
        pltpu.VMEM((M, DM), jnp.bfloat16),
        pltpu.VMEM((NPAIR, RG, 2, 8, 3 * DH), u32),
        pltpu.VMEM((H * DH // 2, DM), u32),
        pltpu.VMEM((S // 2, DM), u32),
        *[pltpu.VMEM((RG, 8, DM), u32)] * 3,
        pltpu.VMEM((16, 2, 2, 8, DM), u32),
        pltpu.VMEM((3, 8, PAD + S, 128), f32),
        pltpu.VMEM((SEG // 2, DM), u32),
        pltpu.VMEM((S // 2, 2 * DM), u32),
        pltpu.VMEM((L, DM), f32),
        pltpu.VMEM((L, H * DH), f32),
        pltpu.VMEM((L, DM), f32),
        pltpu.SemaphoreType.DMA((KT,)),
        pltpu.SemaphoreType.DMA((2 * NB,)),
        pltpu.SemaphoreType.DMA((NB,)),
        pltpu.SemaphoreType.DMA((2 * NB,)),
        pltpu.SemaphoreType.DMA((NB,)),
        pltpu.SemaphoreType.DMA((NSTEP,)),
        pltpu.SemaphoreType.DMA((2,)),
        pltpu.SemaphoreType.DMA((1,)),
    ]
    return kernel, scratch


def pallas_concat_heads__memory_aug_recurrent_mem_tr__sliding_local_dilated__prompt_kernel(
    A_x, A_mem0, A_Wq, A_Wk, A_Wv, A_Wo, A_seg_len, B_x, B_wqkv, B_wo,
):
    B, S, DM = A_x.shape
    H, DH = A_Wq.shape[1], A_Wq.shape[2]
    M = A_mem0.shape[1]
    assert B == 1 and B_x.shape == (1, S, DM)
    kernel, scratch = _make_kernel(S, DM, H, DH, M, int(A_seg_len))
    heads = lambda w: w.reshape(DM // 16, 2, 8, H, DH)
    out = pl.pallas_call(
        kernel,
        out_shape=jax.ShapeDtypeStruct((S, 2 * DM), jnp.bfloat16),
        in_specs=[pl.BlockSpec(memory_space=pl.ANY)] * 9,
        out_specs=pl.BlockSpec(memory_space=pl.ANY),
        scratch_shapes=scratch,
        compiler_params=pltpu.CompilerParams(vmem_limit_bytes=110 * 1024 * 1024),
    )(
        A_x.reshape(S, DM), A_mem0.reshape(M, DM), heads(A_Wq), heads(A_Wk), heads(A_Wv),
        A_Wo.reshape(H * DH, DM), B_x.reshape(S, DM), B_wqkv.reshape(DM // 16, 16, 3 * DM),
        B_wo.reshape(_HB // 16, 2, 8, DM // _HB, DM),
    )
    return out.reshape(1, S, 2 * DM)
```

```python
import functools

import jax
import jax.numpy as jnp
import jax.experimental.pallas as pl
import jax.experimental.pallas.tpu as pltpu

_NT = (((1,), (1,)), ((), ()))
_MASKED = -1000000000.0

_HB, _W, _DIL = 32, 8, 2
_PAD = 16
_TB = 1024
_TS = 256
_WG = 4
_LAG = 19
_TIE = 2
_TAIL = 8
_UNROLL = 4
_TIES = ((32, 0), (96, 0), (32, 512), (96, 512))


def _split(a, b):
    u = jnp.concatenate([a, b], axis=0)
    return (pltpu.bitcast(u.astype(jnp.uint16), jnp.uint32),
            pltpu.bitcast((u >> 16).astype(jnp.uint16), jnp.uint32))


def _bf16(u):
    return pltpu.bitcast(u, jnp.bfloat16)


def _words(x):
    return pltpu.bitcast(x.astype(jnp.bfloat16), jnp.uint32)


def _tie(never, tok, x, r=0, c=0):
    cat = lambda parts, axis: jnp.concatenate([p for p in parts if p.size], axis=axis)
    mid = cat([x[r:r + 8, :c], jnp.where(never, tok, x[r:r + 8, c:c + 128]), x[r:r + 8, c + 128:]], 1)
    return cat([x[:r], mid, x[r + 8:]], 0)


def tile(j):
    return pl.ds(j * 128, 128)


def _rows(i, n):
    return pl.ds(i * n, n) if isinstance(i, int) else pl.ds(pl.multiple_of(i * n, n), n)


def _make_kernel(S, DM, H, DH, M, SEG):
    L = M + SEG
    PAD, W, DIL, TB, TS, WG = _PAD, _W, _DIL, _TB, _TS, _WG
    NB = S // TB
    NPAIR = H // 2
    UN = _UNROLL
    NSTEP = S // SEG // UN
    RG = DM // 16
    KT = DM // 128
    PPI = NPAIR // (2 * NB)
    DPI = 16 // NB
    GPI = RG // NB
    assert DM == 1024 and DH == 128 and DM // _HB == 32 and NPAIR == 2 * NB * PPI and PAD >= DIL * (W - 1)
    scale_a = DH ** -0.5
    scale_b = (DM // _HB) ** -0.5

    def kernel(xa_hbm, mem_hbm, wq_hbm, wk_hbm, wv_hbm, woa_hbm, xb_hbm, wb_hbm, wob_hbm,
               out_hbm,
               xa, memv, wa, woa, xb, wb0, wb1, wb2, wob, qkv, ob, outs, hbuf, obuf, acc,
               s_wq, s_wb, s_xb, s_pair, s_wob, s_xa, s_misc, s_out):
        u32 = lambda r: r.bitcast(jnp.uint32)
        xa_h, woa_h, xb_h, wb_h, wob_h, out_h = (
            u32(xa_hbm), u32(woa_hbm), u32(xb_hbm), u32(wb_hbm), u32(wob_hbm), u32(out_hbm))
        wa_h = [u32(wq_hbm), u32(wk_hbm), u32(wv_hbm)]
        wb = [wb0, wb1, wb2]

        def cp_first(c):
            n = RG // KT
            return [pltpu.make_async_copy(wb_h.at[pl.ds(c * n, n), :, pl.ds(0, DM)], wb0.at[pl.ds(c * n, n)], s_wq.at[c]),
                    pltpu.make_async_copy(xb_h.at[pl.ds(0, TB // 2), tile(c)], xb.at[pl.ds(0, TB // 2), tile(c)], s_wq.at[c])]

        def cp_wb(m, c):
            return pltpu.make_async_copy(wb_h.at[_rows(c, GPI), :, pl.ds(m * DM, DM)], wb[m].at[_rows(c, GPI)],
                                         s_wb.at[(m - 1) * NB + c])

        def cp_xb(c):
            return pltpu.make_async_copy(xb_h.at[_rows(c, TB // 2)], xb.at[_rows(c, TB // 2)], s_xb.at[c])

        def cp_pair(hp):
            return [pltpu.make_async_copy(wa_h[m].at[:, :, :, hp, :], wa.at[hp, :, :, :, tile(m)], s_pair.at[hp // PPI])
                    for m in range(3)]

        def cp_wob(dp):
            return pltpu.make_async_copy(wob_h.at[:, :, :, dp, :], wob.at[dp], s_wob.at[dp // DPI])

        def cp_woa():
            return pltpu.make_async_copy(woa_h, woa, s_misc.at[0])

        def cp_xa(i):
            return pltpu.make_async_copy(xa_h.at[_rows(i, UN * SEG // 2)], xa.at[_rows(i, UN * SEG // 2)], s_xa.at[i])

        def cp_mem():
            return pltpu.make_async_copy(mem_hbm, memv, s_misc.at[1])

        def cp_out(s):
            n = UN * SEG // 2
            return pltpu.make_async_copy(outs.at[_rows(s, n)], out_h.at[_rows(s, n)], s_out.at[0])

        def start_pairs(q):
            for u in range(PPI):
                for cp in cp_pair(q * PPI + u):
                    cp.start()

        for c in range(KT):
            for cp in cp_first(c):
                cp.start()
        cp_wb(1, 0).start()
        for i in range(1, NB):
            cp_xb(i).start()
            cp_wb(1, i).start()
        for i in range(NB):
            cp_wb(2, i).start()
            start_pairs(i)

        def wait_filled(buf, sem):
            pltpu.make_async_copy(buf, buf, sem).wait()

        lane = jax.lax.broadcasted_iota(jnp.int32, (8, 128), 1)

        last = 32 * (lane & 3) + (lane & 28) + (lane >> 5)

        def exchange(t):
            for b in (1, 2, 4):
                t = [jnp.where((lane & (4 * b)) != 0, t[j ^ b], t[j]) for j in range(8)]
            return t

        def permute(grp, r, pre, gate):
            t = [gate(grp[r, :, tile(j)]) for j in range(8)]
            if pre:
                t = t[:1] + [jnp.take_along_axis(t[j], lane ^ (4 * j), axis=1) for j in range(1, 8)]
            t = [jnp.take_along_axis(u, last ^ (4 * j), axis=1) for j, u in enumerate(exchange(t))]
            for j in range(8):
                grp[r, :, tile(j)] = t[j]
            return t

        def split(ref, idx, gate):
            a, b = _split(gate(ref[idx(0)]), ref[idx(1)])
            ref[idx(0)], ref[idx(1)] = a, b
            return [a, b]

        def first_block():
            same = lambda u: u
            n = RG // KT
            dst = qkv.at[0, :, pl.ds(PAD, TB), :]
            for cp in cp_first(0):
                cp.wait()
            for g in range(n):
                permute(wb0, g, False, same)
            for c in range(KT):
                if c + 1 < KT:
                    for cp in cp_first(c + 1):
                        cp.wait()
                    for g in range(n):
                        permute(wb0, (c + 1) * n + g, False, same)
                else:
                    cp_wb(1, 0).wait()
                    for g in range(GPI):
                        permute(wb1, g, False, same)
                x = _bf16(xb[0:TB // 2, tile(c)])
                for j in range(8):
                    r = jnp.dot(x, _bf16(wb0[c * n:(c + 1) * n, :, tile(j)].reshape(64, 128)),
                                preferred_element_type=jnp.float32)
                    dst[j] = r if c == 0 else dst[j] + r

        def proj_body(m, i, carry):
            if m == 0:
                cp_xb(i).wait()
            elif m == 1:
                for u in range(DPI):
                    cp_wob(i * DPI + u).start()
                start_pairs(NB + i)
            else:
                for u in range(NSTEP // NB):
                    cp_xa(i * (NSTEP // NB) + u).start()
            if m < 2:
                cp_wb(m + 1, i).wait()
                nxt = wb[m + 1].at[_rows(i, GPI)]
            else:
                dims = wob.at[_rows(i, DPI)]
                wait_filled(dims, s_wob.at[i])
            if m > 0:
                pairs = wa.at[_rows((m - 1) * NB + i, PPI)]
                wait_filled(pairs, s_pair.at[(m - 1) * NB + i])

            work = []
            if m < 2:
                work.append([functools.partial(permute, nxt, g, m == 1) for g in range(GPI)])
            else:
                work.append([functools.partial(split, dims, lambda e, u=u, r=r, c=c: (u, r, e, slice(None), tile(c)))
                             for u in range(DPI) for r in range(2) for c in range(8)])
            if m > 0:
                work.append([functools.partial(split, pairs, lambda e, u=u, g=g, c=c: (u, g, e, slice(None), tile(c)))
                             for u in range(PPI) for g in range(RG) for c in range(3)])

            dst = qkv.at[m, :, pl.ds(pl.multiple_of(PAD + i * TB, 8), TB), :]
            never = (i + lane) < 0
            gate = lambda u: u
            slots = [(j, t) for j in range(8) for t in range(0, TB, TS)]
            for n, (j, t) in enumerate(slots):
                x = xb[pl.ds(pl.multiple_of(i * (TB // 2) + t // 2, TS // 2), TS // 2), :]
                for a, at in enumerate(_TIES):
                    part, parts = n * len(_TIES) + a, len(slots) * len(_TIES)
                    done = [u for jobs in work
                            for job in jobs[part * len(jobs) // parts:(part + 1) * len(jobs) // parts]
                            for u in job(gate)]
                    if done:
                        x = _tie(never, functools.reduce(jnp.bitwise_or, done), x, *at)
                r = jnp.dot(_bf16(x), _bf16(wb[m][:, :, tile(j)].reshape(DM // 2, 128)),
                            preferred_element_type=jnp.float32)
                dst[j, t:t + TS, :] = r
                gate = functools.partial(jnp.where, never, pltpu.bitcast(r[0:8], jnp.uint32))
            return carry

        first_block()
        for m in range(3):
            if m == 2:
                cp_woa().start()
                cp_mem().start()
            jax.lax.fori_loop(1 if m == 0 else 0, NB, functools.partial(proj_body, m), 0)

        cp_mem().wait()
        cp_woa().wait()
        for m in (1, 2):
            for j in range(8):
                qkv[m, j, 0:PAD, :] = jnp.broadcast_to(qkv[m, j, PAD:PAD + 1, :], (PAD, 128))
        hbuf[0:M, :] = memv[...].astype(jnp.float32)

        row = jax.lax.broadcasted_iota(jnp.int32, (L, 128), 0)
        col = jax.lax.broadcasted_iota(jnp.int32, (L, 128), 1)
        sub = jax.lax.broadcasted_iota(jnp.int32, (8, 128), 0)

        def window_pieces(s, never):
            near = qkv.at[:, :, pl.ds(pl.multiple_of(s * SEG, SEG), PAD + SEG), :]
            st = {}

            def gate(a, tok):
                return jnp.where(never, tok, a)

            def win(m, j, g, w):
                return near[m, j, pl.ds(PAD + g * 8 - DIL * w, 8), :]

            def qk(g, half, tok):
                accs = st.setdefault(("acc", g), [None] * W)
                for j in range(4 * half, 4 * half + 4):
                    qj = gate(win(0, j, g, 0), tok)
                    for w in range(W):
                        p = qj * win(1, j, g, w)
                        accs[w] = p if accs[w] is None else accs[w] + p
                if half == 0:
                    return functools.reduce(jnp.add, accs)
                else:
                    lg = []
                    for w in range(W):
                        a = accs[w]
                        a = a + pltpu.roll(a, 64, 1)
                        a = a + pltpu.roll(a, 32, 1)
                        a = a * scale_b
                        if g * 8 < DIL * w:
                            a = jnp.where(s * SEG + g * 8 + sub >= DIL * w, a, _MASKED)
                        lg.append(a)
                    top = functools.reduce(jnp.maximum, lg)
                    es = [jnp.exp(a - top) for a in lg]
                    st["e", g] = es
                    st["inv", g] = 1.0 / functools.reduce(jnp.add, es)
                    return st["inv", g]

            def pv(g, half, tok):
                inv = gate(st["inv", g], tok)
                ps = [e * inv for e in st["e", g]]
                done = []
                for j in range(4 * half, 4 * half + 4):
                    st["o", g, j] = functools.reduce(jnp.add, [ps[w] * win(2, j, g, w) for w in range(W)])
                    done.append(st["o", g, j])
                    if g % 2 == 1:
                        both = jnp.concatenate([st.pop(("o", g - 1, j)), st.pop(("o", g, j))], axis=0)
                        ob[(g // 2) * 8:(g // 2) * 8 + 8, j * 128:(j + 1) * 128] = _words(both)
                return functools.reduce(jnp.add, done)

            return [functools.partial(fn, g, half)
                    for g in range(SEG // 8) for fn, half in ((qk, 0), (qk, 1), (pv, 0), (pv, 1))]

        def step(s):
            hbuf[M:L, :] = _bf16(xa[_rows(s, SEG // 2), :]).astype(jnp.float32)
            allowed = (row < M) | (row >= col)
            real = col < L
            zpad = jnp.zeros((128 - L, DH), jnp.float32)
            out = outs.at[_rows(s, SEG // 2)]
            never = (s + sub) < 0
            pieces = window_pieces(s, never)
            qs, ks, vs, es, ls = {}, {}, {}, {}, {}

            def project_in(h, done):
                x = hbuf[...] if done is None else _tie(never, done, hbuf[...])
                r = jnp.dot(x, _bf16(wa[h // 2, :, h % 2].reshape(DM // 2, 3 * DH)), preferred_element_type=jnp.float32)
                qs[h] = r[:, 0:DH]
                ks[h] = jnp.concatenate([r[:, DH:2 * DH], zpad], axis=0).astype(jnp.bfloat16)
                vs[h] = jnp.concatenate([r[:, 2 * DH:3 * DH], zpad], axis=0).astype(jnp.bfloat16)
                return r[0:8, 0:DH]

            def scores(h):
                sc = jax.lax.dot_general(qs.pop(h), ks.pop(h), _NT, preferred_element_type=jnp.float32) * scale_a
                sc = jnp.where(allowed, sc, _MASKED)
                sc = jnp.where(real, sc, -jnp.inf)
                e = jnp.exp(sc - jnp.max(sc, axis=1, keepdims=True))
                es[h] = e
                ls[h] = 1.0 / jnp.sum(e, axis=1, keepdims=True)

            def values(h):
                obuf[:, h * DH:(h + 1) * DH] = jnp.dot(
                    es.pop(h), vs.pop(h), preferred_element_type=jnp.float32) * ls.pop(h)

            def project_out(h):
                r = jnp.dot(obuf[:, h * DH:(h + WG) * DH], _bf16(woa[h * DH // 2:(h + WG) * DH // 2, :]),
                            preferred_element_type=jnp.float32)
                if h == 0:
                    acc[...] = r
                elif h + WG < H:
                    acc[...] += r
                else:
                    r = r + acc[...]
                    hbuf[0:M, :] = r[0:M]
                    out[:, 0:DM] = _words(r[M:L])

            def window_out(j):
                w = jnp.concatenate([wob[dp, r, e, :, tile(j)] for dp in range(16) for e in range(2) for r in range(2)], axis=0)
                r = jnp.dot(_bf16(ob[...]), _bf16(w), preferred_element_type=jnp.float32)
                out[:, DM + j * 128:DM + (j + 1) * 128] = _words(r)

            nxt = 0
            done = {}
            for h in range(H):
                tok = project_in(h, done.pop(h, None))
                if pieces:
                    done[h + _TIE] = pieces.pop(0)(tok)
                if h >= 1:
                    scores(h - 1)
                if h >= 2:
                    values(h - 2)
                if h >= _LAG and (h - _LAG) % WG == 0:
                    project_out(nxt)
                    nxt += WG
            if _TAIL == 0:
                for j in range(0, 4):
                    window_out(j)
                scores(H - 1)
                values(H - 2)
                while nxt < H - 2 * WG:
                    project_out(nxt)
                    nxt += WG
                for j in range(4, 8):
                    window_out(j)
                values(H - 1)
                project_out(H - 2 * WG)
                project_out(H - WG)
            else:
                while nxt < H - 3 * WG:
                    project_out(nxt)
                    nxt += WG
                scores(H - 1)
                values(H - 2)
                project_out(H - 3 * WG)
                for j in range(0, 8 - _TAIL):
                    window_out(j)
                values(H - 1)
                project_out(H - 2 * WG)
                project_out(H - WG)
                for j in range(8 - _TAIL, 8):
                    window_out(j)

        def seg_body(i, carry):
            cp_xa(i).wait()
            for u in range(UN):
                step(i * UN + u)
            cp_out(i).start()
            return carry

        jax.lax.fori_loop(0, NSTEP, seg_body, 0)
        pltpu.make_async_copy(outs, out_h, s_out.at[0]).wait()

    f32, u32 = jnp.float32, jnp.uint32
    scratch = [
        pltpu.VMEM((S // 2, DM), u32),
        pltpu.VMEM((M, DM), jnp.bfloat16),
        pltpu.VMEM((NPAIR, RG, 2, 8, 3 * DH), u32),
        pltpu.VMEM((H * DH // 2, DM), u32),
        pltpu.VMEM((S // 2, DM), u32),
        *[pltpu.VMEM((RG, 8, DM), u32)] * 3,
        pltpu.VMEM((16, 2, 2, 8, DM), u32),
        pltpu.VMEM((3, 8, PAD + S, 128), f32),
        pltpu.VMEM((SEG // 2, DM), u32),
        pltpu.VMEM((S // 2, 2 * DM), u32),
        pltpu.VMEM((L, DM), f32),
        pltpu.VMEM((L, H * DH), f32),
        pltpu.VMEM((L, DM), f32),
        pltpu.SemaphoreType.DMA((KT,)),
        pltpu.SemaphoreType.DMA((2 * NB,)),
        pltpu.SemaphoreType.DMA((NB,)),
        pltpu.SemaphoreType.DMA((2 * NB,)),
        pltpu.SemaphoreType.DMA((NB,)),
        pltpu.SemaphoreType.DMA((NSTEP,)),
        pltpu.SemaphoreType.DMA((2,)),
        pltpu.SemaphoreType.DMA((1,)),
    ]
    return kernel, scratch


def pallas_concat_heads__memory_aug_recurrent_mem_tr__sliding_local_dilated__prompt_kernel(
    A_x, A_mem0, A_Wq, A_Wk, A_Wv, A_Wo, A_seg_len, B_x, B_wqkv, B_wo,
):
    B, S, DM = A_x.shape
    H, DH = A_Wq.shape[1], A_Wq.shape[2]
    M = A_mem0.shape[1]
    assert B == 1 and B_x.shape == (1, S, DM)
    kernel, scratch = _make_kernel(S, DM, H, DH, M, int(A_seg_len))
    heads = lambda w: w.reshape(DM // 16, 2, 8, H, DH)
    out = pl.pallas_call(
        kernel,
        out_shape=jax.ShapeDtypeStruct((S, 2 * DM), jnp.bfloat16),
        in_specs=[pl.BlockSpec(memory_space=pl.ANY)] * 9,
        out_specs=pl.BlockSpec(memory_space=pl.ANY),
        scratch_shapes=scratch,
        compiler_params=pltpu.CompilerParams(vmem_limit_bytes=110 * 1024 * 1024),
    )(
        A_x.reshape(S, DM), A_mem0.reshape(M, DM), heads(A_Wq), heads(A_Wk), heads(A_Wv),
        A_Wo.reshape(H * DH, DM), B_x.reshape(S, DM), B_wqkv.reshape(DM // 16, 16, 3 * DM),
        B_wo.reshape(_HB // 16, 2, 8, DM // _HB, DM),
    )
    return out.reshape(1, S, 2 * DM)
```

```python
import functools

import jax
import jax.numpy as jnp
import jax.experimental.pallas as pl
import jax.experimental.pallas.tpu as pltpu

_NT = (((1,), (1,)), ((), ()))
_MASKED = -1000000000.0

_HB, _W, _DIL = 32, 8, 2
_PAD = 16
_TB = 1024
_TS = 256
_WG = 4
_LAG = 19
_TIE = 2
_TAIL = 8
_UNROLL = 4
_ARRIVED = (1, 3, 4, 6, 6, 9, 9, 9)
_TIES = ((32, 0), (96, 0), (32, 512), (96, 512))


def _split(a, b):
    u = jnp.concatenate([a, b], axis=0)
    return (pltpu.bitcast(u.astype(jnp.uint16), jnp.uint32),
            pltpu.bitcast((u >> 16).astype(jnp.uint16), jnp.uint32))


def _bf16(u):
    return pltpu.bitcast(u, jnp.bfloat16)


def _words(x):
    return pltpu.bitcast(x.astype(jnp.bfloat16), jnp.uint32)


def _tie(never, tok, x, r=0, c=0):
    cat = lambda parts, axis: jnp.concatenate([p for p in parts if p.size], axis=axis)
    mid = cat([x[r:r + 8, :c], jnp.where(never, tok, x[r:r + 8, c:c + 128]), x[r:r + 8, c + 128:]], 1)
    return cat([x[:r], mid, x[r + 8:]], 0)


def tile(j):
    return pl.ds(j * 128, 128)


def _rows(i, n):
    return pl.ds(i * n, n) if isinstance(i, int) else pl.ds(pl.multiple_of(i * n, n), n)


def _make_kernel(S, DM, H, DH, M, SEG):
    L = M + SEG
    PAD, W, DIL, TB, TS, WG = _PAD, _W, _DIL, _TB, _TS, _WG
    NB = S // TB
    NPAIR = H // 2
    UN = _UNROLL
    NSTEP = S // SEG // UN
    RG = DM // 16
    KT = DM // 128
    PPI = NPAIR // (2 * NB)
    DPI = 16 // NB
    GPI = RG // NB
    assert DM == 1024 and DH == 128 and DM // _HB == 32 and NPAIR == 2 * NB * PPI and PAD >= DIL * (W - 1)
    scale_a = DH ** -0.5
    scale_b = (DM // _HB) ** -0.5

    def kernel(xa_hbm, mem_hbm, wq_hbm, wk_hbm, wv_hbm, woa_hbm, xb_hbm, wb_hbm, wob_hbm,
               out_hbm,
               xa, memv, wa, woa, xb, wb0, wb1, wb2, wob, qkv, ob, outs, hbuf, obuf, acc,
               s_wq, s_wb, s_xb, s_pair, s_wob, s_xa, s_misc, s_out):
        u32 = lambda r: r.bitcast(jnp.uint32)
        xa_h, woa_h, xb_h, wb_h, wob_h, out_h = (
            u32(xa_hbm), u32(woa_hbm), u32(xb_hbm), u32(wb_hbm), u32(wob_hbm), u32(out_hbm))
        wa_h = [u32(wq_hbm), u32(wk_hbm), u32(wv_hbm)]
        wb = [wb0, wb1, wb2]

        def cp_first(c):
            n = RG // KT
            return [pltpu.make_async_copy(wb_h.at[pl.ds(c * n, n), :, pl.ds(0, DM)], wb0.at[pl.ds(c * n, n)], s_wq.at[c]),
                    pltpu.make_async_copy(xb_h.at[pl.ds(0, TB // 2), tile(c)], xb.at[pl.ds(0, TB // 2), tile(c)], s_wq.at[c])]

        def cp_wb(m, c):
            return pltpu.make_async_copy(wb_h.at[_rows(c, GPI), :, pl.ds(m * DM, DM)], wb[m].at[_rows(c, GPI)],
                                         s_wb.at[(m - 1) * NB + c])

        def cp_xb(c):
            return pltpu.make_async_copy(xb_h.at[_rows(c, TB // 2)], xb.at[_rows(c, TB // 2)], s_xb.at[c])

        def cp_pair(hp):
            return [pltpu.make_async_copy(wa_h[m].at[:, :, :, hp, :], wa.at[hp, :, :, :, tile(m)], s_pair.at[hp // PPI])
                    for m in range(3)]

        def cp_wob(dp):
            return pltpu.make_async_copy(wob_h.at[:, :, :, dp, :], wob.at[dp], s_wob.at[dp // DPI])

        def cp_woa():
            return pltpu.make_async_copy(woa_h, woa, s_misc.at[0])

        def cp_xa(i):
            return pltpu.make_async_copy(xa_h.at[_rows(i, UN * SEG // 2)], xa.at[_rows(i, UN * SEG // 2)], s_xa.at[i])

        def cp_mem():
            return pltpu.make_async_copy(mem_hbm, memv, s_misc.at[1])

        def cp_out(s):
            n = UN * SEG // 2
            return pltpu.make_async_copy(outs.at[_rows(s, n)], out_h.at[_rows(s, n)], s_out.at[0])

        def start_pairs(q):
            for u in range(PPI):
                for cp in cp_pair(q * PPI + u):
                    cp.start()

        for c in range(KT):
            for cp in cp_first(c):
                cp.start()
        cp_wb(1, 0).start()
        for i in range(1, NB):
            cp_xb(i).start()
            cp_wb(1, i).start()
        for i in range(NB):
            cp_wb(2, i).start()
            start_pairs(i)

        def wait_filled(buf, sem):
            pltpu.make_async_copy(buf, buf, sem).wait()

        lane = jax.lax.broadcasted_iota(jnp.int32, (8, 128), 1)

        last = 32 * (lane & 3) + (lane & 28) + (lane >> 5)

        def exchange(t):
            for b in (1, 2, 4):
                t = [jnp.where((lane & (4 * b)) != 0, t[j ^ b], t[j]) for j in range(8)]
            return t

        def permute(grp, r, pre, gate):
            t = [gate(grp[r, :, tile(j)]) for j in range(8)]
            if pre:
                t = t[:1] + [jnp.take_along_axis(t[j], lane ^ (4 * j), axis=1) for j in range(1, 8)]
            t = [jnp.take_along_axis(u, last ^ (4 * j), axis=1) for j, u in enumerate(exchange(t))]
            for j in range(8):
                grp[r, :, tile(j)] = t[j]
            return t

        def split(ref, idx, gate):
            a, b = _split(gate(ref[idx(0)]), ref[idx(1)])
            ref[idx(0)], ref[idx(1)] = a, b
            return [a, b]

        def first_block():
            n = RG // KT
            dst = qkv.at[0, :, pl.ds(PAD, TB), :]
            arrived = ready = 0

            def prepare(upto):
                nonlocal ready
                for c in range(ready, upto):
                    for g in range(n if c < KT else GPI):
                        permute(wb[c // KT], c % KT * n + g, False, lambda u: u)
                ready = max(ready, upto)

            for c in range(KT):
                for a in range(arrived, _ARRIVED[c]):
                    for cp in (cp_first(a) if a < KT else [cp_wb(1, 0)]):
                        cp.wait()
                arrived = max(arrived, _ARRIVED[c])
                prepare(min(c + 2, arrived))
                x = _bf16(xb[0:TB // 2, tile(c)])
                for j in range(8):
                    r = jnp.dot(x, _bf16(wb0[c * n:(c + 1) * n, :, tile(j)].reshape(64, 128)),
                                preferred_element_type=jnp.float32)
                    dst[j] = r if c == 0 else dst[j] + r

        def proj_body(m, i, carry):
            if m == 0:
                cp_xb(i).wait()
            elif m == 1:
                for u in range(DPI):
                    cp_wob(i * DPI + u).start()
                start_pairs(NB + i)
            else:
                for u in range(NSTEP // NB):
                    cp_xa(i * (NSTEP // NB) + u).start()
            if m < 2:
                cp_wb(m + 1, i).wait()
                nxt = wb[m + 1].at[_rows(i, GPI)]
            else:
                dims = wob.at[_rows(i, DPI)]
                wait_filled(dims, s_wob.at[i])
            if m > 0:
                pairs = wa.at[_rows((m - 1) * NB + i, PPI)]
                wait_filled(pairs, s_pair.at[(m - 1) * NB + i])

            work = []
            if m < 2:
                work.append([functools.partial(permute, nxt, g, m == 1) for g in range(GPI)])
            else:
                work.append([functools.partial(split, dims, lambda e, u=u, r=r, c=c: (u, r, e, slice(None), tile(c)))
                             for u in range(DPI) for r in range(2) for c in range(8)])
            if m > 0:
                work.append([functools.partial(split, pairs, lambda e, u=u, g=g, c=c: (u, g, e, slice(None), tile(c)))
                             for u in range(PPI) for g in range(RG) for c in range(3)])

            dst = qkv.at[m, :, pl.ds(pl.multiple_of(PAD + i * TB, 8), TB), :]
            never = (i + lane) < 0
            gate = lambda u: u
            slots = [(j, t) for j in range(8) for t in range(0, TB, TS)]
            for n, (j, t) in enumerate(slots):
                x = xb[pl.ds(pl.multiple_of(i * (TB // 2) + t // 2, TS // 2), TS // 2), :]
                for a, at in enumerate(_TIES):
                    part, parts = n * len(_TIES) + a, len(slots) * len(_TIES)
                    done = [u for jobs in work
                            for job in jobs[part * len(jobs) // parts:(part + 1) * len(jobs) // parts]
                            for u in job(gate)]
                    if done:
                        x = _tie(never, functools.reduce(jnp.bitwise_or, done), x, *at)
                r = jnp.dot(_bf16(x), _bf16(wb[m][:, :, tile(j)].reshape(DM // 2, 128)),
                            preferred_element_type=jnp.float32)
                dst[j, t:t + TS, :] = r
                gate = functools.partial(jnp.where, never, pltpu.bitcast(r[0:8], jnp.uint32))
            return carry

        first_block()
        for m in range(3):
            if m == 2:
                cp_woa().start()
                cp_mem().start()
            jax.lax.fori_loop(1 if m == 0 else 0, NB, functools.partial(proj_body, m), 0)

        cp_mem().wait()
        cp_woa().wait()
        for m in (1, 2):
            for j in range(8):
                qkv[m, j, 0:PAD, :] = jnp.broadcast_to(qkv[m, j, PAD:PAD + 1, :], (PAD, 128))
        hbuf[0:M, :] = memv[...].astype(jnp.float32)

        row = jax.lax.broadcasted_iota(jnp.int32, (L, 128), 0)
        col = jax.lax.broadcasted_iota(jnp.int32, (L, 128), 1)
        sub = jax.lax.broadcasted_iota(jnp.int32, (8, 128), 0)

        def window_pieces(s, never):
            near = qkv.at[:, :, pl.ds(pl.multiple_of(s * SEG, SEG), PAD + SEG), :]
            st = {}

            def gate(a, tok):
                return jnp.where(never, tok, a)

            def win(m, j, g, w):
                return near[m, j, pl.ds(PAD + g * 8 - DIL * w, 8), :]

            def qk(g, half, tok):
                accs = st.setdefault(("acc", g), [None] * W)
                for j in range(4 * half, 4 * half + 4):
                    qj = gate(win(0, j, g, 0), tok)
                    for w in range(W):
                        p = qj * win(1, j, g, w)
                        accs[w] = p if accs[w] is None else accs[w] + p
                if half == 0:
                    return functools.reduce(jnp.add, accs)
                else:
                    lg = []
                    for w in range(W):
                        a = accs[w]
                        a = a + pltpu.roll(a, 64, 1)
                        a = a + pltpu.roll(a, 32, 1)
                        a = a * scale_b
                        if g * 8 < DIL * w:
                            a = jnp.where(s * SEG + g * 8 + sub >= DIL * w, a, _MASKED)
                        lg.append(a)
                    top = functools.reduce(jnp.maximum, lg)
                    es = [jnp.exp(a - top) for a in lg]
                    st["e", g] = es
                    st["inv", g] = 1.0 / functools.reduce(jnp.add, es)
                    return st["inv", g]

            def pv(g, half, tok):
                inv = gate(st["inv", g], tok)
                ps = [e * inv for e in st["e", g]]
                done = []
                for j in range(4 * half, 4 * half + 4):
                    st["o", g, j] = functools.reduce(jnp.add, [ps[w] * win(2, j, g, w) for w in range(W)])
                    done.append(st["o", g, j])
                    if g % 2 == 1:
                        both = jnp.concatenate([st.pop(("o", g - 1, j)), st.pop(("o", g, j))], axis=0)
                        ob[(g // 2) * 8:(g // 2) * 8 + 8, j * 128:(j + 1) * 128] = _words(both)
                return functools.reduce(jnp.add, done)

            return [functools.partial(fn, g, half)
                    for g in range(SEG // 8) for fn, half in ((qk, 0), (qk, 1), (pv, 0), (pv, 1))]

        def step(s):
            hbuf[M:L, :] = _bf16(xa[_rows(s, SEG // 2), :]).astype(jnp.float32)
            allowed = (row < M) | (row >= col)
            real = col < L
            zpad = jnp.zeros((128 - L, DH), jnp.float32)
            out = outs.at[_rows(s, SEG // 2)]
            never = (s + sub) < 0
            pieces = window_pieces(s, never)
            qs, ks, vs, es, ls = {}, {}, {}, {}, {}

            def project_in(h, done):
                x = hbuf[...] if done is None else _tie(never, done, hbuf[...])
                r = jnp.dot(x, _bf16(wa[h // 2, :, h % 2].reshape(DM // 2, 3 * DH)), preferred_element_type=jnp.float32)
                qs[h] = r[:, 0:DH]
                ks[h] = jnp.concatenate([r[:, DH:2 * DH], zpad], axis=0).astype(jnp.bfloat16)
                vs[h] = jnp.concatenate([r[:, 2 * DH:3 * DH], zpad], axis=0).astype(jnp.bfloat16)
                return r[0:8, 0:DH]

            def scores(h):
                sc = jax.lax.dot_general(qs.pop(h), ks.pop(h), _NT, preferred_element_type=jnp.float32) * scale_a
                sc = jnp.where(allowed, sc, _MASKED)
                sc = jnp.where(real, sc, -jnp.inf)
                e = jnp.exp(sc - jnp.max(sc, axis=1, keepdims=True))
                es[h] = e
                ls[h] = 1.0 / jnp.sum(e, axis=1, keepdims=True)

            def values(h):
                obuf[:, h * DH:(h + 1) * DH] = jnp.dot(
                    es.pop(h), vs.pop(h), preferred_element_type=jnp.float32) * ls.pop(h)

            def project_out(h):
                r = jnp.dot(obuf[:, h * DH:(h + WG) * DH], _bf16(woa[h * DH // 2:(h + WG) * DH // 2, :]),
                            preferred_element_type=jnp.float32)
                if h == 0:
                    acc[...] = r
                elif h + WG < H:
                    acc[...] += r
                else:
                    r = r + acc[...]
                    hbuf[0:M, :] = r[0:M]
                    out[:, 0:DM] = _words(r[M:L])

            def window_out(j):
                w = jnp.concatenate([wob[dp, r, e, :, tile(j)] for dp in range(16) for e in range(2) for r in range(2)], axis=0)
                r = jnp.dot(_bf16(ob[...]), _bf16(w), preferred_element_type=jnp.float32)
                out[:, DM + j * 128:DM + (j + 1) * 128] = _words(r)

            nxt = 0
            done = {}
            for h in range(H):
                tok = project_in(h, done.pop(h, None))
                if pieces:
                    done[h + _TIE] = pieces.pop(0)(tok)
                if h >= 1:
                    scores(h - 1)
                if h >= 2:
                    values(h - 2)
                if h >= _LAG and (h - _LAG) % WG == 0:
                    project_out(nxt)
                    nxt += WG
            if _TAIL == 0:
                for j in range(0, 4):
                    window_out(j)
                scores(H - 1)
                values(H - 2)
                while nxt < H - 2 * WG:
                    project_out(nxt)
                    nxt += WG
                for j in range(4, 8):
                    window_out(j)
                values(H - 1)
                project_out(H - 2 * WG)
                project_out(H - WG)
            else:
                while nxt < H - 3 * WG:
                    project_out(nxt)
                    nxt += WG
                scores(H - 1)
                values(H - 2)
                project_out(H - 3 * WG)
                for j in range(0, 8 - _TAIL):
                    window_out(j)
                values(H - 1)
                project_out(H - 2 * WG)
                project_out(H - WG)
                for j in range(8 - _TAIL, 8):
                    window_out(j)

        def seg_body(i, carry):
            cp_xa(i).wait()
            for u in range(UN):
                step(i * UN + u)
            cp_out(i).start()
            return carry

        jax.lax.fori_loop(0, NSTEP, seg_body, 0)
        pltpu.make_async_copy(outs, out_h, s_out.at[0]).wait()

    f32, u32 = jnp.float32, jnp.uint32
    scratch = [
        pltpu.VMEM((S // 2, DM), u32),
        pltpu.VMEM((M, DM), jnp.bfloat16),
        pltpu.VMEM((NPAIR, RG, 2, 8, 3 * DH), u32),
        pltpu.VMEM((H * DH // 2, DM), u32),
        pltpu.VMEM((S // 2, DM), u32),
        *[pltpu.VMEM((RG, 8, DM), u32)] * 3,
        pltpu.VMEM((16, 2, 2, 8, DM), u32),
        pltpu.VMEM((3, 8, PAD + S, 128), f32),
        pltpu.VMEM((SEG // 2, DM), u32),
        pltpu.VMEM((S // 2, 2 * DM), u32),
        pltpu.VMEM((L, DM), f32),
        pltpu.VMEM((L, H * DH), f32),
        pltpu.VMEM((L, DM), f32),
        pltpu.SemaphoreType.DMA((KT,)),
        pltpu.SemaphoreType.DMA((2 * NB,)),
        pltpu.SemaphoreType.DMA((NB,)),
        pltpu.SemaphoreType.DMA((2 * NB,)),
        pltpu.SemaphoreType.DMA((NB,)),
        pltpu.SemaphoreType.DMA((NSTEP,)),
        pltpu.SemaphoreType.DMA((2,)),
        pltpu.SemaphoreType.DMA((1,)),
    ]
    return kernel, scratch


def pallas_concat_heads__memory_aug_recurrent_mem_tr__sliding_local_dilated__prompt_kernel(
    A_x, A_mem0, A_Wq, A_Wk, A_Wv, A_Wo, A_seg_len, B_x, B_wqkv, B_wo,
):
    B, S, DM = A_x.shape
    H, DH = A_Wq.shape[1], A_Wq.shape[2]
    M = A_mem0.shape[1]
    assert B == 1 and B_x.shape == (1, S, DM)
    kernel, scratch = _make_kernel(S, DM, H, DH, M, int(A_seg_len))
    heads = lambda w: w.reshape(DM // 16, 2, 8, H, DH)
    out = pl.pallas_call(
        kernel,
        out_shape=jax.ShapeDtypeStruct((S, 2 * DM), jnp.bfloat16),
        in_specs=[pl.BlockSpec(memory_space=pl.ANY)] * 9,
        out_specs=pl.BlockSpec(memory_space=pl.ANY),
        scratch_shapes=scratch,
        compiler_params=pltpu.CompilerParams(vmem_limit_bytes=110 * 1024 * 1024),
    )(
        A_x.reshape(S, DM), A_mem0.reshape(M, DM), heads(A_Wq), heads(A_Wk), heads(A_Wv),
        A_Wo.reshape(H * DH, DM), B_x.reshape(S, DM), B_wqkv.reshape(DM // 16, 16, 3 * DM),
        B_wo.reshape(_HB // 16, 2, 8, DM // _HB, DM),
    )
    return out.reshape(1, S, 2 * DM)
```

```python
import functools

import jax
import jax.numpy as jnp
import jax.experimental.pallas as pl
import jax.experimental.pallas.tpu as pltpu

_NT = (((1,), (1,)), ((), ()))
_MASKED = -1000000000.0

_HB, _W, _DIL = 32, 8, 2
_PAD = 16

_TB = 1024
_TS = 256
_ARRIVED = (1, 3, 4, 6, 6, 9, 9, 9)
_TIES = ((32, 0), (96, 0), (32, 512), (96, 512))
_UNROLL = 4
_WG = 4
_TIE = 2


def _bf16(u):
    return pltpu.bitcast(u, jnp.bfloat16)


def _words(x):
    return pltpu.bitcast(x.astype(jnp.bfloat16), jnp.uint32)


def _split(a, b):
    u = jnp.concatenate([a, b], axis=0)
    return (pltpu.bitcast(u.astype(jnp.uint16), jnp.uint32),
            pltpu.bitcast((u >> 16).astype(jnp.uint16), jnp.uint32))


def _tile(j):
    return pl.ds(j * 128, 128)


def _rows(i, n):
    return pl.ds(i * n, n) if isinstance(i, int) else pl.ds(pl.multiple_of(i * n, n), n)


def _gate(never, tok, x):
    return jnp.where(never, tok, x)


def _tie(never, tok, x, r=0, c=0):
    cat = lambda parts, axis: jnp.concatenate([p for p in parts if p.size], axis=axis)
    mid = cat([x[r:r + 8, :c], _gate(never, tok, x[r:r + 8, c:c + 128]), x[r:r + 8, c + 128:]], 1)
    return cat([x[:r], mid, x[r + 8:]], 0)


def _make_kernel(S, DM, H, DH, M, SEG):
    L = M + SEG
    PAD, W, DIL, TB, TS, UN, WG = _PAD, _W, _DIL, _TB, _TS, _UNROLL, _WG
    NB = S // TB
    NSTEP = S // SEG // UN
    NPAIR = H // 2
    RG = DM // 16
    KT = DM // 128
    GPI = RG // NB
    PPI = NPAIR // (2 * NB)
    DPI = 16 // NB
    assert DM == 1024 and DH == 128 and DM // _HB == 32 and PAD >= DIL * (W - 1)
    assert S == NB * TB == NSTEP * UN * SEG and NPAIR == 2 * NB * PPI and M == 8 and SEG % 16 == 0
    scale_a = DH ** -0.5
    scale_b = (DM // _HB) ** -0.5

    def kernel(xa_hbm, mem_hbm, wq_hbm, wk_hbm, wv_hbm, woa_hbm, xb_hbm, wb_hbm, wob_hbm,
               out_hbm,
               xa, memv, wa, woa, xb, wb0, wb1, wb2, wob, qkv, ob, outs, hbuf, obuf, acc,
               s_wq, s_wb, s_xb, s_pair, s_wob, s_xa, s_misc, s_out):
        u32 = lambda r: r.bitcast(jnp.uint32)
        xa_h, woa_h, xb_h, wb_h, wob_h, out_h = (
            u32(xa_hbm), u32(woa_hbm), u32(xb_hbm), u32(wb_hbm), u32(wob_hbm), u32(out_hbm))
        wa_h = [u32(wq_hbm), u32(wk_hbm), u32(wv_hbm)]
        wb = [wb0, wb1, wb2]
        copy = pltpu.make_async_copy

        def cp_first(c):
            n = RG // KT
            return [copy(wb_h.at[_rows(c, n), :, pl.ds(0, DM)], wb0.at[_rows(c, n)], s_wq.at[c]),
                    copy(xb_h.at[pl.ds(0, TB // 2), _tile(c)], xb.at[pl.ds(0, TB // 2), _tile(c)], s_wq.at[c])]

        def cp_wb(m, c):
            return copy(wb_h.at[_rows(c, GPI), :, pl.ds(m * DM, DM)], wb[m].at[_rows(c, GPI)],
                        s_wb.at[(m - 1) * NB + c])

        def cp_xb(c):
            return copy(xb_h.at[_rows(c, TB // 2)], xb.at[_rows(c, TB // 2)], s_xb.at[c])

        def start_pairs(q):
            for u in range(PPI):
                hp = q * PPI + u
                for m in range(3):
                    copy(wa_h[m].at[:, :, :, hp, :], wa.at[hp, :, :, :, _tile(m)], s_pair.at[q]).start()

        def start_dims(q):
            for u in range(DPI):
                dp = q * DPI + u
                copy(wob_h.at[:, :, :, dp, :], wob.at[dp], s_wob.at[q]).start()

        def cp_woa():
            return copy(woa_h, woa, s_misc.at[0])

        def cp_mem():
            return copy(mem_hbm, memv, s_misc.at[1])

        def cp_xa(i):
            return copy(xa_h.at[_rows(i, UN * SEG // 2)], xa.at[_rows(i, UN * SEG // 2)], s_xa.at[i])

        def cp_out(i):
            return copy(outs.at[_rows(i, UN * SEG // 2)], out_h.at[_rows(i, UN * SEG // 2)], s_out.at[0])

        def wait_filled(buf, sem):
            copy(buf, buf, sem).wait()

        for c in range(KT):
            for cp in cp_first(c):
                cp.start()
        cp_wb(1, 0).start()
        for i in range(1, NB):
            cp_xb(i).start()
            cp_wb(1, i).start()
        for i in range(NB):
            cp_wb(2, i).start()
            start_pairs(i)

        lane = jax.lax.broadcasted_iota(jnp.int32, (8, 128), 1)

        def permute(grp, r, pre, gate):
            t = [gate(grp[r, :, _tile(j)]) for j in range(8)]
            if pre:
                t = t[:1] + [jnp.take_along_axis(t[j], lane ^ (4 * j), axis=1) for j in range(1, 8)]
            for b in (1, 2, 4):
                t = [jnp.where((lane & (4 * b)) != 0, t[j ^ b], t[j]) for j in range(8)]
            src = 32 * (lane & 3) + (lane & 28) + (lane >> 5)
            t = [jnp.take_along_axis(t[j], src ^ (4 * j), axis=1) for j in range(8)]
            for j in range(8):
                grp[r, :, _tile(j)] = t[j]
            return t

        def split(ref, u, g, c, gate):
            a, b = _split(gate(ref[u, g, 0, :, _tile(c)]), ref[u, g, 1, :, _tile(c)])
            ref[u, g, 0, :, _tile(c)] = a
            ref[u, g, 1, :, _tile(c)] = b
            return [a, b]

        def first_block():
            n = RG // KT
            dst = qkv.at[0, :, pl.ds(PAD, TB), :]
            arrived = ready = 0
            for c in range(KT):
                for a in range(arrived, _ARRIVED[c]):
                    for cp in (cp_first(a) if a < KT else [cp_wb(1, 0)]):
                        cp.wait()
                arrived = _ARRIVED[c]
                for a in range(ready, min(c + 2, arrived)):
                    for g in range(n if a < KT else GPI):
                        permute(wb[a // KT], a % KT * n + g, False, lambda u: u)
                    ready = a + 1
                x = _bf16(xb[0:TB // 2, _tile(c)])
                for j in range(8):
                    r = jnp.dot(x, _bf16(wb0[c * n:(c + 1) * n, :, _tile(j)].reshape(64, 128)),
                                preferred_element_type=jnp.float32)
                    dst[j] = r if c == 0 else dst[j] + r
            assert arrived == ready == KT + 1

        def proj_body(m, i, carry):
            work = []
            if m == 0:
                cp_xb(i).wait()
            if m == 1:
                start_dims(i)
                start_pairs(NB + i)
            if m == 2:
                for u in range(NSTEP // NB):
                    cp_xa(i * (NSTEP // NB) + u).start()
            if m < 2:
                cp_wb(m + 1, i).wait()
                nxt = wb[m + 1].at[_rows(i, GPI)]
                work.append([functools.partial(permute, nxt, g, m == 1) for g in range(GPI)])
            else:
                dims = wob.at[_rows(i, DPI)]
                wait_filled(dims, s_wob.at[i])
                work.append([functools.partial(split, dims, u, g, c)
                             for u in range(DPI) for g in range(2) for c in range(8)])
            if m > 0:
                pairs = wa.at[_rows((m - 1) * NB + i, PPI)]
                wait_filled(pairs, s_pair.at[(m - 1) * NB + i])
                work.append([functools.partial(split, pairs, u, g, c)
                             for u in range(PPI) for g in range(RG) for c in range(3)])

            dst = qkv.at[m, :, pl.ds(pl.multiple_of(PAD + i * TB, 8), TB), :]
            never = (i + lane) < 0
            gate = lambda u: u
            slots = [(j, t) for j in range(8) for t in range(0, TB, TS)]
            for n, (j, t) in enumerate(slots):
                x = xb[pl.ds(pl.multiple_of(i * (TB // 2) + t // 2, TS // 2), TS // 2), :]
                for a, at in enumerate(_TIES):
                    part, parts = n * len(_TIES) + a, len(slots) * len(_TIES)
                    done = [u for jobs in work
                            for job in jobs[part * len(jobs) // parts:(part + 1) * len(jobs) // parts]
                            for u in job(gate)]
                    if done:
                        x = _tie(never, functools.reduce(jnp.bitwise_or, done), x, *at)
                r = jnp.dot(_bf16(x), _bf16(wb[m][:, :, _tile(j)].reshape(DM // 2, 128)),
                            preferred_element_type=jnp.float32)
                dst[j, t:t + TS, :] = r
                gate = functools.partial(_gate, never, pltpu.bitcast(r[0:8], jnp.uint32))
            return carry

        first_block()
        for m in range(3):
            if m == 2:
                cp_woa().start()
                cp_mem().start()
            jax.lax.fori_loop(1 if m == 0 else 0, NB, functools.partial(proj_body, m), 0)

        cp_mem().wait()
        cp_woa().wait()
        for m in (1, 2):
            for j in range(8):
                qkv[m, j, 0:PAD, :] = jnp.broadcast_to(qkv[m, j, PAD:PAD + 1, :], (PAD, 128))
        hbuf[0:M, :] = memv[...].astype(jnp.float32)

        row = jax.lax.broadcasted_iota(jnp.int32, (L, 128), 0)
        col = jax.lax.broadcasted_iota(jnp.int32, (L, 128), 1)
        sub = jax.lax.broadcasted_iota(jnp.int32, (8, 128), 0)

        def window_pieces(s, never):
            near = qkv.at[:, :, pl.ds(pl.multiple_of(s * SEG, SEG), PAD + SEG), :]
            st = {}

            def win(m, j, g, w):
                return near[m, j, pl.ds(PAD + g * 8 - DIL * w, 8), :]

            def qk(g, half, tok):
                dots = st.setdefault(("qk", g), [None] * W)
                for j in range(4 * half, 4 * half + 4):
                    q = _gate(never, tok, win(0, j, g, 0))
                    for w in range(W):
                        p = q * win(1, j, g, w)
                        dots[w] = p if dots[w] is None else dots[w] + p
                if half == 0:
                    return functools.reduce(jnp.add, dots)
                logits = []
                for w in range(W):
                    a = dots[w]
                    a = a + pltpu.roll(a, 64, 1)
                    a = a + pltpu.roll(a, 32, 1)
                    a = a * scale_b
                    if g * 8 < DIL * w:
                        a = jnp.where(s * SEG + g * 8 + sub >= DIL * w, a, _MASKED)
                    logits.append(a)
                top = functools.reduce(jnp.maximum, logits)
                st["e", g] = [jnp.exp(a - top) for a in logits]
                st["inv", g] = 1.0 / functools.reduce(jnp.add, st["e", g])
                return st["inv", g]

            def pv(g, half, tok):
                inv = _gate(never, tok, st["inv", g])
                ps = [e * inv for e in st["e", g]]
                done = []
                for j in range(4 * half, 4 * half + 4):
                    st["o", g, j] = functools.reduce(jnp.add, [ps[w] * win(2, j, g, w) for w in range(W)])
                    done.append(st["o", g, j])
                    if g % 2 == 1:
                        both = jnp.concatenate([st.pop(("o", g - 1, j)), st.pop(("o", g, j))], axis=0)
                        ob[_rows(g // 2, 8), _tile(j)] = _words(both)
                return functools.reduce(jnp.add, done)

            return [functools.partial(fn, g, half)
                    for g in range(SEG // 8) for fn in (qk, pv) for half in (0, 1)]

        def step(s):
            hbuf[M:L, :] = _bf16(xa[_rows(s, SEG // 2), :]).astype(jnp.float32)
            allowed = (row < M) | (row >= col)
            real = col < L
            zpad = jnp.zeros((128 - L, DH), jnp.float32)
            out = outs.at[_rows(s, SEG // 2)]
            never = (s + sub) < 0
            pieces = window_pieces(s, never)
            qs, ks, vs, es, ls = {}, {}, {}, {}, {}

            def project_in(h, done):
                x = hbuf[...] if done is None else _tie(never, done, hbuf[...])
                r = jnp.dot(x, _bf16(wa[h // 2, :, h % 2].reshape(DM // 2, 3 * DH)),
                            preferred_element_type=jnp.float32)
                qs[h] = r[:, 0:DH]
                ks[h] = jnp.concatenate([r[:, DH:2 * DH], zpad], axis=0).astype(jnp.bfloat16)
                vs[h] = jnp.concatenate([r[:, 2 * DH:3 * DH], zpad], axis=0).astype(jnp.bfloat16)
                return r[0:8, 0:DH]

            def scores(h):
                sc = jax.lax.dot_general(qs.pop(h), ks.pop(h), _NT, preferred_element_type=jnp.float32) * scale_a
                sc = jnp.where(allowed, sc, _MASKED)
                sc = jnp.where(real, sc, -jnp.inf)
                e = jnp.exp(sc - jnp.max(sc, axis=1, keepdims=True))
                es[h] = e
                ls[h] = 1.0 / jnp.sum(e, axis=1, keepdims=True)

            def values(h):
                obuf[:, _tile(h)] = jnp.dot(es.pop(h), vs.pop(h), preferred_element_type=jnp.float32) * ls.pop(h)

            def project_out(h):
                r = jnp.dot(obuf[:, h * DH:(h + WG) * DH], _bf16(woa[h * DH // 2:(h + WG) * DH // 2, :]),
                            preferred_element_type=jnp.float32)
                if h == 0:
                    acc[...] = r
                elif h + WG < H:
                    acc[...] += r
                else:
                    r = r + acc[...]
                    hbuf[0:M, :] = r[0:M]
                    out[:, 0:DM] = _words(r[M:L])

            def window_out(j):
                w = jnp.concatenate([wob[dp, g, e, :, _tile(j)]
                                     for dp in range(16) for e in range(2) for g in range(2)], axis=0)
                r = jnp.dot(_bf16(ob[...]), _bf16(w), preferred_element_type=jnp.float32)
                out[:, _tile(KT + j)] = _words(r)

            done = {}
            for h in range(H):
                tok = project_in(h, done.pop(h, None))
                if pieces:
                    done[h + _TIE] = pieces.pop(0)(tok)
                if h >= 1:
                    scores(h - 1)
                if h >= 2:
                    values(h - 2)
                if h % WG == WG - 1 and h >= 5 * WG - 1:
                    project_out(h + 1 - 5 * WG)
            project_out(H - 4 * WG)
            scores(H - 1)
            values(H - 2)
            project_out(H - 3 * WG)
            values(H - 1)
            project_out(H - 2 * WG)
            project_out(H - WG)
            for j in range(KT):
                window_out(j)

        def seg_body(i, carry):
            cp_xa(i).wait()
            for u in range(UN):
                step(i * UN + u)
            cp_out(i).start()
            return carry

        jax.lax.fori_loop(0, NSTEP, seg_body, 0)
        copy(outs, out_h, s_out.at[0]).wait()

    f32, u32 = jnp.float32, jnp.uint32
    scratch = [
        pltpu.VMEM((S // 2, DM), u32),
        pltpu.VMEM((M, DM), jnp.bfloat16),
        pltpu.VMEM((NPAIR, RG, 2, 8, 3 * DH), u32),
        pltpu.VMEM((H * DH // 2, DM), u32),
        pltpu.VMEM((S // 2, DM), u32),
        *[pltpu.VMEM((RG, 8, DM), u32)] * 3,
        pltpu.VMEM((16, 2, 2, 8, DM), u32),
        pltpu.VMEM((3, 8, PAD + S, 128), f32),
        pltpu.VMEM((SEG // 2, DM), u32),
        pltpu.VMEM((S // 2, 2 * DM), u32),
        pltpu.VMEM((L, DM), f32),
        pltpu.VMEM((L, H * DH), f32),
        pltpu.VMEM((L, DM), f32),
        pltpu.SemaphoreType.DMA((KT,)),
        pltpu.SemaphoreType.DMA((2 * NB,)),
        pltpu.SemaphoreType.DMA((NB,)),
        pltpu.SemaphoreType.DMA((2 * NB,)),
        pltpu.SemaphoreType.DMA((NB,)),
        pltpu.SemaphoreType.DMA((NSTEP,)),
        pltpu.SemaphoreType.DMA((2,)),
        pltpu.SemaphoreType.DMA((1,)),
    ]
    return kernel, scratch


def pallas_concat_heads__memory_aug_recurrent_mem_tr__sliding_local_dilated__prompt_kernel(
    A_x, A_mem0, A_Wq, A_Wk, A_Wv, A_Wo, A_seg_len, B_x, B_wqkv, B_wo,
):
    B, S, DM = A_x.shape
    H, DH = A_Wq.shape[1], A_Wq.shape[2]
    M = A_mem0.shape[1]
    assert B == 1 and B_x.shape == (1, S, DM)
    kernel, scratch = _make_kernel(S, DM, H, DH, M, int(A_seg_len))
    heads = lambda w: w.reshape(DM // 16, 2, 8, H, DH)
    out = pl.pallas_call(
        kernel,
        out_shape=jax.ShapeDtypeStruct((S, 2 * DM), jnp.bfloat16),
        in_specs=[pl.BlockSpec(memory_space=pl.ANY)] * 9,
        out_specs=pl.BlockSpec(memory_space=pl.ANY),
        scratch_shapes=scratch,
        compiler_params=pltpu.CompilerParams(vmem_limit_bytes=110 * 1024 * 1024),
    )(
        A_x.reshape(S, DM), A_mem0.reshape(M, DM), heads(A_Wq), heads(A_Wk), heads(A_Wv),
        A_Wo.reshape(H * DH, DM), B_x.reshape(S, DM), B_wqkv.reshape(DM // 16, 16, 3 * DM),
        B_wo.reshape(_HB // 16, 2, 8, DM // _HB, DM),
    )
    return out.reshape(1, S, 2 * DM)
```
